```python
import jax
import jax.numpy as jnp

def _softmax(x, axis=-1):
    return jax.nn.softmax(x, axis=axis)

def _gelu(x):
    return jax.nn.gelu(x, approximate=True)

def _silu(x):
    return jax.nn.silu(x)

def _sigmoid(x):
    return jax.nn.sigmoid(x)

def _layernorm(x, axis=-1, eps=1e-05):
    m = jnp.mean(x, axis=axis, keepdims=True)
    v = jnp.var(x, axis=axis, keepdims=True)
    return (x - m) / jnp.sqrt(v + eps)

def _scatter_add(tgt, idx, src, axis=0):
    return tgt.at[idx].add(src)

def _segment_sum(src, seg, n):
    return jax.ops.segment_sum(src, seg, n)

class _Rng:

    def __init__(self, key):
        self._k = key

    def _next(self):
        self._k, sub = jax.random.split(self._k)
        return sub

    def normal(self, shape):
        return jax.random.normal(self._next(), shape, dtype=jnp.bfloat16)

    def randint(self, lo, hi, shape):
        return jax.random.randint(self._next(), shape, lo, hi, dtype=jnp.int32)

    def uniform(self, shape, lo=0.0, hi=1.0):
        return jax.random.uniform(self._next(), shape, jnp.bfloat16, lo, hi)

    def permutation(self, n):
        return jax.random.permutation(self._next(), n)
kernel_name = 'sequential_preLN__memory_aug_recurrent_mem_tr__moe_arch_mod__prompt'

def setup_inputs():
    _rng = _Rng(jax.random.key(int.from_bytes(__import__("os").urandom(4), "little")))
    _w = lambda a: (lambda t: t.astype(jnp.bfloat16) if jnp.issubdtype(t.dtype, jnp.floating) else t)(jnp.asarray(a))

    def _A_setup():
        B, S, Dm = (1, 2048, 512)
        H, Dh = (32, 128)
        M, seg = (8, 32)
        seg = min(seg, S)
        S = S // seg * seg
        return {'x': _w((lambda *s: _rng.normal(s) * 0.05)(B, S, Dm)), 'mem0': _w((lambda *s: _rng.normal(s) * 0.05)(B, M, Dm)), 'Wq': _w((lambda *s: _rng.normal(s) * 0.05)(Dm, H, Dh) * Dm ** (-0.5)), 'Wk': _w((lambda *s: _rng.normal(s) * 0.05)(Dm, H, Dh) * Dm ** (-0.5)), 'Wv': _w((lambda *s: _rng.normal(s) * 0.05)(Dm, H, Dh) * Dm ** (-0.5)), 'Wo': _w((lambda *s: _rng.normal(s) * 0.05)(H, Dh, Dm) * (H * Dh) ** (-0.5)), 'seg_len': seg}
    _A_in = _A_setup()

    def _B_setup():
        B, S, D, F, C = (1, 2048, 512, 1792, 2)
        return {'x': _w((lambda *s: _rng.normal(s) * 0.05)(B, S, D)), 'w_r': _w((lambda *s: _rng.normal(s) * 0.05)(D)), 'w_gate': _w((lambda *s: _rng.normal(s) * 0.05)(D, F)), 'w_up': _w((lambda *s: _rng.normal(s) * 0.05)(D, F)), 'w_down': _w((lambda *s: _rng.normal(s) * 0.05)(F, D))}
    _B_in = _B_setup()
    return {'A_x': _A_in['x'], 'A_mem0': _A_in['mem0'], 'A_Wq': _A_in['Wq'], 'A_Wk': _A_in['Wk'], 'A_Wv': _A_in['Wv'], 'A_Wo': _A_in['Wo'], 'A_seg_len': _A_in['seg_len'], 'B_x': _B_in['x'], 'B_w_r': _B_in['w_r'], 'B_w_gate': _B_in['w_gate'], 'B_w_up': _B_in['w_up'], 'B_w_down': _B_in['w_down']}

def reference(A_x, A_mem0, A_Wq, A_Wk, A_Wv, A_Wo, A_seg_len, B_x, B_w_r, B_w_gate, B_w_up, B_w_down):

    def _A_ref(x, mem0, Wq, Wk, Wv, Wo, seg_len):
        B, S, Dm = x.shape
        H, Dh = (Wq.shape[1], Wq.shape[2])
        M = mem0.shape[1]
        scale = Dh ** (-0.5)
        n_seg = S // seg_len
        L = M + seg_len
        idx = jnp.arange(L)
        mask = (idx[:, None] < M) | (idx[:, None] >= idx[None, :])
        mem = mem0
        outs = []
        for s in range(n_seg):
            xs = x[:, s * seg_len:(s + 1) * seg_len, :].copy()
            h = jnp.concatenate([mem, xs], axis=1)
            q = jnp.einsum('btd,dhe->bhte', h, Wq)
            k = jnp.einsum('btd,dhe->bhte', h, Wk)
            v = jnp.einsum('btd,dhe->bhte', h, Wv)
            scores = jnp.einsum('bhqe,bhke->bhqk', q, k) * scale
            scores = jnp.where(mask[None, None], scores, -1000000000.0)
            p = _softmax(scores, axis=-1)
            o = jnp.einsum('bhqk,bhke->bhqe', p, v)
            o = jnp.einsum('bhte,hed->btd', o, Wo)
            mem = o[:, :M, :].copy()
            outs.append(o[:, M:, :])
        return jnp.concatenate(outs, axis=1)

    def _B_ref(x, w_r, w_gate, w_up, w_down):
        B, S, D = x.shape
        C = 2
        r = x @ w_r
        idx = jnp.argsort(-r, axis=-1)[:, :C]
        idx_e = jnp.repeat(idx.reshape(B, C, 1), D, axis=2)
        x_sel = jnp.take_along_axis(x, idx_e, axis=1)
        g = _silu(x_sel @ w_gate)
        u = x_sel @ w_up
        y = g * u @ w_down
        r_sel = _sigmoid(jnp.take_along_axis(r, idx, axis=1))
        y = y * r_sel.reshape(B, C, 1)
        b_off = (jnp.arange(B) * S).reshape(B, 1)
        flat_idx = (idx + b_off).reshape(B * C)
        zero = (x * 0.0).reshape(B * S, D)
        upd = _scatter_add(zero, flat_idx, y.reshape(B * C, D), axis=0)
        return x + upd.reshape(B, S, D)
    x = A_x
    h = x + _A_ref(_layernorm(x, axis=-1), A_mem0, A_Wq, A_Wk, A_Wv, A_Wo, A_seg_len)
    h2 = h + _B_ref(_layernorm(h, axis=-1), B_w_r, B_w_gate, B_w_up, B_w_down)
    return h2
```

```python
import functools

import jax
import jax.numpy as jnp
import numpy as np
from jax import lax
import jax.experimental.pallas as pl
import jax.experimental.pallas.tpu as pltpu

F32 = jnp.float32
BF16 = jnp.bfloat16
U32 = jnp.uint32

_LANES = 128
_PRE = 8
_TOP = 2
_UNROLL = 2
_LOOKAHEAD = 3


def _mm(a, b):
    return lax.dot_general(a, b, (((1,), (0,)), ((), ())), preferred_element_type=F32)


def _mm_t(a, b):
    return lax.dot_general(a, b, (((1,), (1,)), ((), ())), preferred_element_type=F32)


def _rnd(x):
    return x.astype(BF16).astype(F32)


def _layernorm(x):
    inv_n = 1.0 / x.shape[-1]
    mean = jnp.sum(x, axis=-1, keepdims=True) * inv_n
    c = x - mean
    var = jnp.sum(c * c, axis=-1, keepdims=True) * inv_n
    eps = float(np.asarray(1e-5, dtype=BF16))
    den = _rnd(jnp.sqrt(_rnd(_rnd(var) + eps)))
    return _rnd(_rnd(x - _rnd(mean)) / den)


def _mxu_order(n_heads, cost_a, lat_ab=200, lat_bc=480, lat_cd=200, defer=28):
    ops, done = [], {}
    t = a = b = c = d = 0
    while d < n_heads:
        d_ready = d < c and t >= done["C", d] + lat_cd
        if c < b and t >= done["B", c] + lat_bc:
            t += 10
            ops.append(("C", c))
            done["C", c] = t
            c += 1
        elif b < a and t >= done["A", b] + lat_ab:
            t += 10
            ops.append(("B", b))
            done["B", b] = t
            b += 1
        elif a < n_heads and not (d_ready and a - d > defer):
            t += cost_a
            ops.append(("A", a))
            done["A", a] = t
            a += 1
        elif d_ready:
            t += 40
            ops.append(("D", d))
            d += 1
        else:
            t += 10
    return ops


def _kernel(
    x_hbm, mem0_ref, wq_hbm, wk_hbm, wv_hbm, wo_hbm, wr_ref, wg_hbm, wu_hbm, wd_hbm,
    out_hbm,
    x_ref, xpre_ref, lhs_ref, stage_ref, w_ref, wo_ref, wg_ref, wu_ref, wd_ref,
    kv_ref, h_ref, out_ref, w_sem, sem,
):
    n_seg, seg, d_model = x_hbm.shape
    n_mem = mem0_ref.shape[0]
    n_heads, d_head = wo_hbm.shape[0], wo_hbm.shape[1]
    n_pairs = n_heads // 2
    n_tiles = d_model // _LANES
    n_rows = seg + n_mem
    scale = float(np.asarray(d_head ** -0.5, dtype=BF16))

    w_words = [w.bitcast(U32) for w in (wq_hbm, wk_hbm, wv_hbm)]

    def pair_copies(i):
        return [
            pltpu.make_async_copy(w_words[m].at[:, i, :], stage_ref.at[m, i], w_sem.at[m * n_pairs + i])
            for m in (1, 2, 0)
        ]

    xpre_copy = pltpu.make_async_copy(x_hbm.at[:, pl.ds(seg - _PRE, _PRE), :], xpre_ref, sem.at[0])
    x_copy = pltpu.make_async_copy(x_hbm, x_ref, sem.at[1])
    wo_copy = pltpu.make_async_copy(wo_hbm.bitcast(U32), wo_ref, sem.at[2])
    ffn_copies = [
        pltpu.make_async_copy(wg_hbm.bitcast(U32), wg_ref, sem.at[3]),
        pltpu.make_async_copy(wu_hbm.bitcast(U32), wu_ref, sem.at[4]),
        pltpu.make_async_copy(wd_hbm.bitcast(U32), wd_ref, sem.at[5]),
    ]
    out_sem = sem.at[6]

    def split_pair(i):
        for c in pair_copies(i):
            c.wait()
        for m in range(3):
            even = stage_ref[m, i, pl.ds(0, d_model // 2, stride=2), :]
            odd = stage_ref[m, i, pl.ds(1, d_model // 2, stride=2), :]
            w_ref[m, 2 * i] = (even & np.uint32(0xFFFF)) | (odd << 16)
            w_ref[m, 2 * i + 1] = (even >> 16) | (odd & np.uint32(0xFFFF0000))

    def project_pre(i):
        lhs = pltpu.bitcast(lhs_ref[...], BF16)
        for m in (1, 2):
            for j in range(2):
                kv_ref[m - 1, 2 * i + j] = _mm(lhs, pltpu.bitcast(w_ref[m, 2 * i + j], BF16))

    xpre_copy.start()
    for i in range(_LOOKAHEAD):
        for c in pair_copies(i):
            c.start()
    xpre_copy.wait()
    xpre = xpre_ref[...].astype(F32).reshape(n_seg * _PRE, d_model)
    lhs_ref[...] = pltpu.bitcast(_layernorm(xpre).astype(BF16), U32)
    split_pair(0)

    def pre_body(i, _):
        @pl.when(i + _LOOKAHEAD < n_pairs)
        def _():
            for c in pair_copies(i + _LOOKAHEAD):
                c.start()

        @pl.when(i == 4)
        def _():
            x_copy.start()

        @pl.when(i + _LOOKAHEAD == n_pairs)
        def _():
            wo_copy.start()

        split_pair(i + 1)
        project_pre(i)

    lax.fori_loop(0, n_pairs - 1, pre_body, None)
    project_pre(n_pairs - 1)
    x_copy.wait()
    wo_copy.wait()
    for c in ffn_copies:
        c.start()

    row = lax.broadcasted_iota(jnp.int32, (n_rows, n_rows), 0)
    col = lax.broadcasted_iota(jnp.int32, (n_rows, n_rows), 1)
    visible = (row >= seg) | (col >= seg) | (row >= col)
    lane = lax.broadcasted_iota(jnp.int32, (seg, _LANES), 1)
    w_route = wr_ref[...].astype(F32)
    order = _mxu_order(n_heads, cost_a=n_rows + 2 * (n_rows - _PRE))

    def route_score(hn):
        prod = hn[:, :_LANES] * w_route[0:1]
        for j in range(1, n_tiles):
            prod = prod + hn[:, j * _LANES:(j + 1) * _LANES] * w_route[j:j + 1]
        return _rnd(jnp.sum(prod, axis=-1, keepdims=True))

    def finish_segment(s, attn, scores):
        h = _rnd(x_ref[s].astype(F32) + _rnd(attn))
        hn = _layernorm(h)
        h_ref[s] = h
        out_ref[s] = (h + hn).astype(BF16)
        return jnp.where(lane == s, route_score(hn), scores)

    def attend(s, xn, mem):
        rows_q = jnp.concatenate([xn, mem], axis=0)
        rows_kv = jnp.concatenate([xn[:seg - _PRE], mem], axis=0)
        pre = pl.ds(pl.multiple_of(s * _PRE, _PRE), _PRE)

        def keys_or_values(m, t):
            y = _mm(rows_kv, pltpu.bitcast(w_ref[m, t], BF16))
            y = jnp.concatenate([y[:seg - _PRE], kv_ref[m - 1, t, pre, :], y[seg - _PRE:]], axis=0)
            return y.astype(BF16)

        q, k, v, p, o = {}, {}, {}, {}, {}
        acc = [None] * n_tiles
        for kind, t in order:
            if kind == "A":
                q[t] = _mm(rows_q, pltpu.bitcast(w_ref[0, t], BF16))
                k[t] = keys_or_values(1, t)
                v[t] = keys_or_values(2, t)
            elif kind == "B":
                sc = jnp.where(visible, _mm_t(q[t], k[t]) * scale, -1e9)
                e = jnp.exp(sc - jnp.max(sc, axis=-1, keepdims=True))
                p[t] = e / jnp.sum(e, axis=-1, keepdims=True)
            elif kind == "C":
                y = _mm(p[t], v[t])
                o[t] = jnp.concatenate([y[seg:], y[:seg]], axis=0)
            else:
                for j in range(n_tiles):
                    w = pltpu.bitcast(wo_ref[t, :, j * _LANES:(j + 1) * _LANES], BF16)
                    y = _mm(o[t], w)
                    acc[j] = y if acc[j] is None else acc[j] + y
        y = jnp.concatenate(acc, axis=1)
        return _rnd(y[:n_mem]), y[n_mem:]

    def seg_body(it, carry):
        mem, xn, attn, scores = carry

        @pl.when(it >= 2)
        def _():
            blk = pl.ds((it - 2) * _UNROLL, _UNROLL)
            pltpu.make_async_copy(out_ref.at[blk], out_hbm.at[blk], out_sem).start()

        for u in range(_UNROLL):
            s = it * _UNROLL + u
            scores = finish_segment((s + n_seg - 1) % n_seg, attn, scores)
            xn_next = _layernorm(x_ref[jnp.minimum(s + 1, n_seg - 1)].astype(F32))
            mem, attn = attend(s, xn, mem)
            xn = xn_next
        return mem, xn, attn, scores

    n_iter = n_seg // _UNROLL
    carry = (
        mem0_ref[...].astype(F32),
        _layernorm(x_ref[0].astype(F32)),
        jnp.zeros((seg, d_model), F32),
        jnp.full((seg, _LANES), -jnp.inf, F32),
    )
    _, _, attn, scores = lax.fori_loop(0, n_iter, seg_body, carry)
    scores = finish_segment(n_seg - 1, attn, scores)
    blk = pl.ds((n_iter - 2) * _UNROLL, 2 * _UNROLL)
    pltpu.make_async_copy(out_ref.at[blk], out_hbm.at[blk], out_sem).start()

    token = lane * seg + lax.broadcasted_iota(jnp.int32, (seg, _LANES), 0)
    live = lane < n_seg
    key = jnp.where(scores == scores, scores, -jnp.inf)
    picks = []
    for _ in range(_TOP):
        best = jnp.max(jnp.where(live, key, -jnp.inf), keepdims=True)
        first = jnp.min(jnp.where(live & (key == best), token, n_seg * seg).astype(F32))
        first = jnp.minimum(first.astype(jnp.int32), n_seg * seg - 1)
        live = live & (token != first)
        picks.append(first)

    slot = lax.broadcasted_iota(jnp.int32, (8, d_model), 0)
    h_sel = jnp.broadcast_to(h_ref[picks[0] // seg, pl.ds(picks[0] % seg, 1), :], (8, d_model))
    for n in range(1, _TOP):
        h_sel = jnp.where(slot == n, h_ref[picks[n] // seg, pl.ds(picks[n] % seg, 1), :], h_sel)
    hn_sel = _layernorm(h_sel)
    for c in ffn_copies:
        c.wait()
    gate = _rnd(_mm(hn_sel, pltpu.bitcast(wg_ref[...], BF16)))
    up = _rnd(_mm(hn_sel, pltpu.bitcast(wu_ref[...], BF16)))
    act = _rnd(_rnd(gate * jax.nn.sigmoid(gate)) * up)
    y = _rnd(_mm(act, pltpu.bitcast(wd_ref[...], BF16)))
    y = _rnd(y * _rnd(jax.nn.sigmoid(route_score(hn_sel))))
    new_rows = h_sel + _rnd(hn_sel + y)

    pltpu.make_async_copy(out_ref, out_hbm, out_sem).wait()
    seg_row = lax.broadcasted_iota(jnp.int32, (seg, d_model), 0)
    for n in range(_TOP):
        s = picks[n] // seg
        old = out_ref[s].astype(F32)
        out_ref[s] = jnp.where(seg_row == picks[n] % seg, new_rows[n:n + 1], old).astype(BF16)
    s0, s1 = picks[0] // seg, picks[1] // seg
    fix0 = pltpu.make_async_copy(out_ref.at[s0], out_hbm.at[s0], sem.at[7])
    fix1 = pltpu.make_async_copy(out_ref.at[s1], out_hbm.at[s1], sem.at[8])
    fix0.start()

    @pl.when(s0 != s1)
    def _():
        fix1.start()
        fix1.wait()

    fix0.wait()


@functools.partial(jax.jit, static_argnames=("A_seg_len",))
def pallas_sequential_preLN__memory_aug_recurrent_mem_tr__moe_arch_mod__prompt_kernel(
    A_x: jax.Array,
    A_mem0: jax.Array,
    A_Wq: jax.Array,
    A_Wk: jax.Array,
    A_Wv: jax.Array,
    A_Wo: jax.Array,
    A_seg_len: int,
    B_x: jax.Array,
    B_w_r: jax.Array,
    B_w_gate: jax.Array,
    B_w_up: jax.Array,
    B_w_down: jax.Array,
):
    del B_x
    batch, seq, d_model = A_x.shape
    n_mem = A_mem0.shape[1]
    _, n_heads, d_head = A_Wq.shape
    d_ff = B_w_gate.shape[1]
    seg = int(A_seg_len)
    n_seg = seq // seg
    assert batch == 1 and seq == n_seg * seg and n_seg <= _LANES and n_seg % _UNROLL == 0

    hbm = pl.BlockSpec(memory_space=pl.ANY)
    vmem = pl.BlockSpec(memory_space=pltpu.VMEM)
    out = pl.pallas_call(
        _kernel,
        out_shape=jax.ShapeDtypeStruct((n_seg, seg, d_model), A_x.dtype),
        in_specs=[hbm, vmem, hbm, hbm, hbm, hbm, vmem, hbm, hbm, hbm],
        out_specs=hbm,
        scratch_shapes=[
            pltpu.VMEM((n_seg, seg, d_model), BF16),
            pltpu.VMEM((n_seg, _PRE, d_model), BF16),
            pltpu.VMEM((n_seg * _PRE // 2, d_model), U32),
            pltpu.VMEM((3, n_heads // 2, d_model, d_head), U32),
            pltpu.VMEM((3, n_heads, d_model // 2, d_head), U32),
            pltpu.VMEM((n_heads, d_head // 2, d_model), U32),
            pltpu.VMEM((d_model // 2, d_ff), U32),
            pltpu.VMEM((d_model // 2, d_ff), U32),
            pltpu.VMEM((d_ff // 2, d_model), U32),
            pltpu.VMEM((2, n_heads, n_seg * _PRE, d_head), F32),
            pltpu.VMEM((n_seg, seg, d_model), F32),
            pltpu.VMEM((n_seg, seg, d_model), BF16),
            pltpu.SemaphoreType.DMA((3 * n_heads // 2,)),
            pltpu.SemaphoreType.DMA((9,)),
        ],
        compiler_params=pltpu.CompilerParams(vmem_limit_bytes=100 * 1024 * 1024),
        name="rmt_mod",
    )(
        A_x.reshape(n_seg, seg, d_model),
        A_mem0.reshape(n_mem, d_model),
        A_Wq, A_Wk, A_Wv, A_Wo,
        B_w_r.reshape(d_model // _LANES, _LANES),
        B_w_gate, B_w_up, B_w_down,
    )
    return out.reshape(batch, seq, d_model)
```

```python
import functools

import jax
import jax.numpy as jnp
import numpy as np
from jax import lax
import jax.experimental.pallas as pl
import jax.experimental.pallas.tpu as pltpu

F32 = jnp.float32
BF16 = jnp.bfloat16
U32 = jnp.uint32

_LANES = 128
_EPS = 1e-5
_PRE = 8
_TOP = 2
_UNROLL = 4
_BATCHES = (0, 1, 3, 7, 12, 16)


def _mm(a, b):
    return lax.dot_general(a, b, (((1,), (0,)), ((), ())), preferred_element_type=F32)


def _mm_t(a, b):
    return lax.dot_general(a, b, (((1,), (1,)), ((), ())), preferred_element_type=F32)


def _rnd(x):
    return x.astype(BF16).astype(F32)


def _moments(x):
    inv_n = 1.0 / x.shape[-1]
    mean = jnp.sum(x, axis=-1, keepdims=True) * inv_n
    c = x - mean
    return mean, c, jnp.sum(c * c, axis=-1, keepdims=True) * inv_n


def _layernorm(x):
    _, c, var = _moments(x)
    return c * lax.rsqrt(var + _EPS)


def _layernorm_rounded(x):
    mean, _, var = _moments(x)
    den = _rnd(jnp.sqrt(_rnd(_rnd(var) + float(np.asarray(_EPS, dtype=BF16)))))
    return _rnd(_rnd(x - _rnd(mean)) / den)


def _issue_order(n_heads, cost_a, lat_ab=200, lat_bc=480, lat_cd=200, defer=28, group=2):
    cost = dict(A=cost_a, B=10, C=10, D=40)
    width = dict(A=1, B=group, C=group, D=1)
    wait = dict(B=("A", lat_ab), C=("B", lat_bc), D=("C", lat_cd))
    nxt = dict.fromkeys(cost, 0)
    ops, done, t = [], {}, 0

    def ready(kind):
        src, lat = wait[kind]
        last = nxt[kind] + width[kind] - 1
        return last < nxt[src] and t >= done[src, last] + lat

    while nxt["D"] < n_heads:
        kind = next((c for c in "CB" if ready(c)), None)
        if kind is None and ready("D") and (nxt["A"] == n_heads or nxt["A"] - nxt["D"] > defer):
            kind = "D"
        if kind is None and nxt["A"] < n_heads:
            kind = "A"
        if kind is None:
            t += 10
            continue
        for _ in range(width[kind]):
            t += cost[kind]
            ops.append((kind, nxt[kind]))
            done[kind, nxt[kind]] = t
            nxt[kind] += 1
    return ops


def _kernel(
    x_hbm, mem0_hbm, wq_hbm, wk_hbm, wv_hbm, wo_hbm, wr_hbm, wg_hbm, wu_hbm, wd_hbm,
    out_hbm,
    mem0_ref, wr_ref, x_ref, xpre_ref, lhs_ref, stage_ref, w_ref, wo_ref, wg_ref, wu_ref, wd_ref,
    kv_ref, attn_ref, h_ref, out_ref, w_sem, sem,
):
    n_seg, seg, d_model = x_hbm.shape
    n_mem = mem0_ref.shape[0]
    n_heads, d_head = wo_hbm.shape[0], wo_hbm.shape[1]
    n_pairs = n_heads // 2
    n_tiles = d_model // _LANES
    n_rows = seg + n_mem
    scale = float(np.asarray(d_head ** -0.5, dtype=BF16))

    w_words = [w.bitcast(U32) for w in (wq_hbm, wk_hbm, wv_hbm)]

    def pair_copy(m, i):
        return pltpu.make_async_copy(
            w_words[m].at[:, i, :], stage_ref.at[m, i], w_sem.at[m * n_pairs + i])

    half = n_seg // 2
    head = _UNROLL + 1
    xpre_copies = [
        pltpu.make_async_copy(
            x_hbm.at[pl.ds(n * half, half), pl.ds(seg - _PRE, _PRE), :],
            xpre_ref.at[pl.ds(n * half, half)], sem.at[n])
        for n in range(2)
    ]
    early_copies = [
        pltpu.make_async_copy(x_hbm.at[pl.ds(0, head)], x_ref.at[pl.ds(0, head)], sem.at[2]),
        pltpu.make_async_copy(mem0_hbm, mem0_ref, sem.at[3]),
        pltpu.make_async_copy(wr_hbm, wr_ref, sem.at[4]),
        pltpu.make_async_copy(wo_hbm.bitcast(U32), wo_ref, sem.at[5]),
    ]
    x_copy = pltpu.make_async_copy(
        x_hbm.at[pl.ds(head, n_seg - head)], x_ref.at[pl.ds(head, n_seg - head)], sem.at[6])
    ffn_copies = [
        pltpu.make_async_copy(wg_hbm.bitcast(U32), wg_ref, sem.at[7]),
        pltpu.make_async_copy(wu_hbm.bitcast(U32), wu_ref, sem.at[8]),
        pltpu.make_async_copy(wd_hbm.bitcast(U32), wd_ref, sem.at[9]),
    ]
    out_sem = sem.at[10]

    bounds = [n_pairs * n // 16 for n in _BATCHES]
    phases = [[(m, i) for i in range(lo, hi) for m in (1, 2)] for lo, hi in zip(bounds, bounds[1:])]
    phases[-1] += [(0, i) for i in range(n_pairs)]
    batches = [[pair_copy(m, i) for m, i in ph] for ph in phases]
    batches += [early_copies, [x_copy] + ffn_copies]

    def split_pair(m, i):
        even = stage_ref[m, i, pl.ds(0, d_model // 2, stride=2), :]
        odd = stage_ref[m, i, pl.ds(1, d_model // 2, stride=2), :]
        w_ref[m, 2 * i] = (even & np.uint32(0xFFFF)) | (odd << 16)
        w_ref[m, 2 * i + 1] = (even >> 16) | (odd & np.uint32(0xFFFF0000))

    for c in xpre_copies:
        c.start()
    for n, c in enumerate(xpre_copies):
        c.wait()
        for nxt in batches[n]:
            nxt.start()
        xpre = xpre_ref[pl.ds(n * half, half)].astype(F32).reshape(half * _PRE, d_model)
        lhs_ref[pl.ds(n * half * _PRE // 2, half * _PRE // 2), :] = pltpu.bitcast(
            _layernorm(xpre).astype(BF16), U32)
    for n, phase in enumerate(phases):
        for c in batches[n]:
            c.wait()
        for c in batches[n + 2]:
            c.start()
        for m, i in phase:
            split_pair(m, i)
            for t in ((2 * i, 2 * i + 1) if m else ()):
                lhs = pltpu.bitcast(lhs_ref[...], BF16)
                kv_ref[(m - 1) * n_heads + t] = _mm(lhs, pltpu.bitcast(w_ref[m, t], BF16))
    for c in early_copies:
        c.wait()

    row = lax.broadcasted_iota(jnp.int32, (n_rows, n_rows), 0)
    col = lax.broadcasted_iota(jnp.int32, (n_rows, n_rows), 1)
    visible = (row >= seg) | (col >= seg) | (row >= col)
    lane = lax.broadcasted_iota(jnp.int32, (seg, _LANES), 1)
    w_route = wr_ref[...].astype(F32)
    order = _issue_order(n_heads, cost_a=n_rows + 2 * (n_rows - _PRE))
    at = order.index(("A", 4))
    order[at:at] = [("F", 0), ("N", 0)]

    def route_score(hn):
        prod = hn[:, :_LANES] * w_route[0:1]
        for j in range(1, n_tiles):
            prod = prod + hn[:, j * _LANES:(j + 1) * _LANES] * w_route[j:j + 1]
        return _rnd(jnp.sum(prod, axis=-1, keepdims=True))

    state = kv_ref.at[2 * n_heads]
    scores_at = pl.ds(n_tiles * seg, seg)

    def stage_segment(s):
        xn = _layernorm(x_ref[s].astype(F32))
        for j in range(n_tiles):
            state[pl.ds(j * seg, seg), :] = xn[:, j * _LANES:(j + 1) * _LANES]

    def finish_segment(s):
        h = _rnd(x_ref[s].astype(F32) + _rnd(attn_ref[...]))
        hn = _layernorm_rounded(h)
        h_ref[s] = h
        out_ref[s] = (h + hn).astype(BF16)
        state[scores_at, :] = jnp.where(lane == s, route_score(hn), state[scores_at, :])

    def attend(s, mem):
        xn = jnp.concatenate([state[pl.ds(j * seg, seg), :] for j in range(n_tiles)], axis=1)
        rows_q = jnp.concatenate([xn, mem], axis=0)
        rows_kv = jnp.concatenate([xn[:seg - _PRE], mem], axis=0)
        pre = pl.ds(pl.multiple_of(s * _PRE, _PRE), _PRE)

        def keys_or_values(m, t):
            y = _mm(rows_kv, pltpu.bitcast(w_ref[m, t], BF16))
            y = jnp.concatenate([y[:seg - _PRE], kv_ref[(m - 1) * n_heads + t, pre, :], y[seg - _PRE:]], axis=0)
            return y.astype(BF16)

        q, k, v, p, o = {}, {}, {}, {}, {}
        acc = [None] * n_tiles
        for kind, t in order:
            if kind == "A":
                q[t] = _mm(rows_q, pltpu.bitcast(w_ref[0, t], BF16))
                k[t] = keys_or_values(1, t)
                v[t] = keys_or_values(2, t)
            elif kind == "B":
                sc = jnp.where(visible, _mm_t(q[t], k[t]) * scale, -1e9)
                e = jnp.exp(sc - jnp.max(sc, axis=-1, keepdims=True))
                p[t] = e / jnp.sum(e, axis=-1, keepdims=True)
            elif kind == "C":
                y = _mm(p[t], v[t])
                o[t] = jnp.concatenate([y[seg:], y[:seg]], axis=0)
            elif kind == "F":
                finish_segment((s + n_seg - 1) % n_seg)
            elif kind == "N":
                stage_segment(jnp.minimum(s + 1, n_seg - 1))
            else:
                for j in range(n_tiles):
                    w = pltpu.bitcast(wo_ref[t, :, j * _LANES:(j + 1) * _LANES], BF16)
                    y = _mm(o[t], w)
                    acc[j] = y if acc[j] is None else acc[j] + y
        y = jnp.concatenate(acc, axis=1)
        attn_ref[...] = y[n_mem:]
        return _rnd(y[:n_mem])

    def seg_body(it, mem):
        @pl.when(it == 1)
        def _():
            x_copy.wait()

        @pl.when(it >= 2)
        def _():
            blk = pl.ds((it - 2) * _UNROLL, _UNROLL)
            pltpu.make_async_copy(out_ref.at[blk], out_hbm.at[blk], out_sem).start()

        for u in range(_UNROLL):
            mem = attend(it * _UNROLL + u, mem)
        return mem

    n_iter = n_seg // _UNROLL
    stage_segment(0)
    attn_ref[...] = jnp.zeros((seg, d_model), F32)
    state[scores_at, :] = jnp.full((seg, _LANES), -jnp.inf, F32)
    lax.fori_loop(0, n_iter, seg_body, mem0_ref[...].astype(F32))
    finish_segment(n_seg - 1)
    scores = state[scores_at, :]
    blk = pl.ds((n_iter - 2) * _UNROLL, 2 * _UNROLL)
    pltpu.make_async_copy(out_ref.at[blk], out_hbm.at[blk], out_sem).start()

    token = lane * seg + lax.broadcasted_iota(jnp.int32, (seg, _LANES), 0)
    live = lane < n_seg
    key = jnp.where(scores == scores, scores, -jnp.inf)
    picks = []
    for _ in range(_TOP):
        best = jnp.max(jnp.where(live, key, -jnp.inf), keepdims=True)
        first = jnp.min(jnp.where(live & (key == best), token, n_seg * seg).astype(F32))
        first = jnp.minimum(first.astype(jnp.int32), n_seg * seg - 1)
        live = live & (token != first)
        picks.append(first)

    slot = lax.broadcasted_iota(jnp.int32, (8, d_model), 0)
    h_sel = jnp.broadcast_to(h_ref[picks[0] // seg, pl.ds(picks[0] % seg, 1), :], (8, d_model))
    for n in range(1, _TOP):
        h_sel = jnp.where(slot == n, h_ref[picks[n] // seg, pl.ds(picks[n] % seg, 1), :], h_sel)
    hn_sel = _layernorm_rounded(h_sel)
    for c in ffn_copies:
        c.wait()
    gate = _rnd(_mm(hn_sel, pltpu.bitcast(wg_ref[...], BF16)))
    up = _rnd(_mm(hn_sel, pltpu.bitcast(wu_ref[...], BF16)))
    act = _rnd(_rnd(gate * jax.nn.sigmoid(gate)) * up)
    y = _rnd(_mm(act, pltpu.bitcast(wd_ref[...], BF16)))
    y = _rnd(y * _rnd(jax.nn.sigmoid(route_score(hn_sel))))
    new_rows = h_sel + _rnd(hn_sel + y)

    pltpu.make_async_copy(out_ref, out_hbm, out_sem).wait()
    seg_row = lax.broadcasted_iota(jnp.int32, (seg, d_model), 0)
    for n in range(_TOP):
        s = picks[n] // seg
        old = out_ref[s].astype(F32)
        out_ref[s] = jnp.where(seg_row == picks[n] % seg, new_rows[n:n + 1], old).astype(BF16)
    s0, s1 = picks[0] // seg, picks[1] // seg
    fix0 = pltpu.make_async_copy(out_ref.at[s0], out_hbm.at[s0], sem.at[11])
    fix1 = pltpu.make_async_copy(out_ref.at[s1], out_hbm.at[s1], sem.at[12])
    fix0.start()

    @pl.when(s0 != s1)
    def _():
        fix1.start()
        fix1.wait()

    fix0.wait()


@functools.partial(jax.jit, static_argnames=("A_seg_len",))
def pallas_sequential_preLN__memory_aug_recurrent_mem_tr__moe_arch_mod__prompt_kernel(
    A_x: jax.Array,
    A_mem0: jax.Array,
    A_Wq: jax.Array,
    A_Wk: jax.Array,
    A_Wv: jax.Array,
    A_Wo: jax.Array,
    A_seg_len: int,
    B_x: jax.Array,
    B_w_r: jax.Array,
    B_w_gate: jax.Array,
    B_w_up: jax.Array,
    B_w_down: jax.Array,
):
    del B_x
    batch, seq, d_model = A_x.shape
    n_mem = A_mem0.shape[1]
    _, n_heads, d_head = A_Wq.shape
    d_ff = B_w_gate.shape[1]
    seg = int(A_seg_len)
    n_seg = seq // seg
    assert batch == 1 and seq == n_seg * seg and n_seg <= _LANES and n_seg % _UNROLL == 0

    hbm = pl.BlockSpec(memory_space=pl.ANY)
    out = pl.pallas_call(
        _kernel,
        out_shape=jax.ShapeDtypeStruct((n_seg, seg, d_model), A_x.dtype),
        in_specs=[hbm] * 10,
        out_specs=hbm,
        scratch_shapes=[
            pltpu.VMEM((n_mem, d_model), BF16),
            pltpu.VMEM((d_model // _LANES, _LANES), BF16),
            pltpu.VMEM((n_seg, seg, d_model), BF16),
            pltpu.VMEM((n_seg, _PRE, d_model), BF16),
            pltpu.VMEM((n_seg * _PRE // 2, d_model), U32),
            pltpu.VMEM((3, n_heads // 2, d_model, d_head), U32),
            pltpu.VMEM((3, n_heads, d_model // 2, d_head), U32),
            pltpu.VMEM((n_heads, d_head // 2, d_model), U32),
            pltpu.VMEM((d_model // 2, d_ff), U32),
            pltpu.VMEM((d_model // 2, d_ff), U32),
            pltpu.VMEM((d_ff // 2, d_model), U32),
            pltpu.VMEM((2 * n_heads + 1, n_seg * _PRE, d_head), F32),
            pltpu.VMEM((seg, d_model), F32),
            pltpu.VMEM((n_seg, seg, d_model), F32),
            pltpu.VMEM((n_seg, seg, d_model), BF16),
            pltpu.SemaphoreType.DMA((3 * n_heads // 2,)),
            pltpu.SemaphoreType.DMA((13,)),
        ],
        compiler_params=pltpu.CompilerParams(vmem_limit_bytes=100 * 1024 * 1024),
        name="rmt_mod",
    )(
        A_x.reshape(n_seg, seg, d_model),
        A_mem0.reshape(n_mem, d_model),
        A_Wq, A_Wk, A_Wv, A_Wo,
        B_w_r.reshape(d_model // _LANES, _LANES),
        B_w_gate, B_w_up, B_w_down,
    )
    return out.reshape(batch, seq, d_model)
```

```python
import functools

import jax
import jax.numpy as jnp
import numpy as np
from jax import lax
import jax.experimental.pallas as pl
import jax.experimental.pallas.tpu as pltpu

F32 = jnp.float32
BF16 = jnp.bfloat16
U32 = jnp.uint32

_LANES = 128
_EPS = 1e-5
_PRE = 8
_ROT = 4
_KEY_BASE = 1 << 29
_UNROLL = 4
_BATCHES = (0, 1, 3, 7, 12, 16)


def _mm(a, b):
    return lax.dot_general(a, b, (((1,), (0,)), ((), ())), preferred_element_type=F32)


def _mm_t(a, b):
    return lax.dot_general(a, b, (((1,), (1,)), ((), ())), preferred_element_type=F32)


def _rnd(x):
    return x.astype(BF16).astype(F32)


def _moments(x):
    inv_n = 1.0 / x.shape[-1]
    mean = jnp.sum(x, axis=-1, keepdims=True) * inv_n
    c = x - mean
    return mean, c, jnp.sum(c * c, axis=-1, keepdims=True) * inv_n


def _layernorm(x):
    _, c, var = _moments(x)
    return c * lax.rsqrt(var + _EPS)


def _layernorm_rounded(x):
    mean, _, var = _moments(x)
    den = _rnd(jnp.sqrt(_rnd(_rnd(var) + float(np.asarray(_EPS, dtype=BF16)))))
    return _rnd(_rnd(x - _rnd(mean)) / den)


def _issue_order(n_heads, cost_a, lat_ab=200, lat_bc=480, lat_cd=200, defer=28, group=2):
    cost = dict(A=cost_a, B=10, C=10, D=40)
    width = dict(A=1, B=group, C=group, D=1)
    wait = dict(B=("A", lat_ab), C=("B", lat_bc), D=("C", lat_cd))
    nxt = dict.fromkeys(cost, 0)
    ops, done, t = [], {}, 0

    def ready(kind):
        src, lat = wait[kind]
        last = nxt[kind] + width[kind] - 1
        return last < nxt[src] and t >= done[src, last] + lat

    while nxt["D"] < n_heads:
        kind = next((c for c in "CB" if ready(c)), None)
        if kind is None and ready("D") and (nxt["A"] == n_heads or nxt["A"] - nxt["D"] > defer):
            kind = "D"
        if kind is None and nxt["A"] < n_heads:
            kind = "A"
        if kind is None:
            t += 10
            continue
        for _ in range(width[kind]):
            t += cost[kind]
            ops.append((kind, nxt[kind]))
            done[kind, nxt[kind]] = t
            nxt[kind] += 1
    return ops


def _kernel(
    x_hbm, mem0_hbm, wq_hbm, wk_hbm, wv_hbm, wo_hbm, wr_hbm, wg_hbm, wu_hbm, wd_hbm,
    out_hbm,
    mem0_ref, wr_ref, x_ref, xpre_ref, lhs_ref, lhs32_ref, stage_ref, w_ref, wo_ref, wg_ref, wu_ref, wd_ref,
    kv_ref, attn_ref, h_ref, hn_ref, out_ref, w_sem, sem,
):
    n_seg, seg, d_model = x_hbm.shape
    n_mem = mem0_ref.shape[0]
    n_heads, d_head = wo_hbm.shape[0], wo_hbm.shape[1]
    n_pairs = n_heads // 2
    n_tiles = d_model // _LANES
    n_rows = seg + n_mem
    scale = float(np.asarray(d_head ** -0.5, dtype=BF16))

    w_words = [w.bitcast(U32) for w in (wq_hbm, wk_hbm, wv_hbm)]

    def pair_copy(m, i):
        return pltpu.make_async_copy(
            w_words[m].at[:, i, :], stage_ref.at[m, i], w_sem.at[m * n_pairs + i])

    slot_of = (2 * n_heads, 0, n_heads)
    half = n_seg // 2
    head = _UNROLL + 1
    xpre_copies = [
        pltpu.make_async_copy(
            x_hbm.at[pl.ds(n * half, half), pl.ds(seg - _PRE, _PRE), :],
            xpre_ref.at[pl.ds(n * half, half)], sem.at[n])
        for n in range(2)
    ]
    early_copies = [
        pltpu.make_async_copy(x_hbm.at[pl.ds(0, head)], x_ref.at[pl.ds(0, head)], sem.at[2]),
        pltpu.make_async_copy(mem0_hbm, mem0_ref, sem.at[3]),
        pltpu.make_async_copy(wr_hbm, wr_ref, sem.at[4]),
    ]
    wo_copy = pltpu.make_async_copy(wo_hbm.bitcast(U32), wo_ref, sem.at[5])
    x_copy = pltpu.make_async_copy(
        x_hbm.at[pl.ds(head, n_seg - head)], x_ref.at[pl.ds(head, n_seg - head)], sem.at[6])
    ffn_copies = [
        pltpu.make_async_copy(wg_hbm.bitcast(U32), wg_ref, sem.at[7]),
        pltpu.make_async_copy(wu_hbm.bitcast(U32), wu_ref, sem.at[8]),
        pltpu.make_async_copy(wd_hbm.bitcast(U32), wd_ref, sem.at[9]),
    ]
    out_sem = sem.at[10]

    bounds = [n_pairs * n // 16 for n in _BATCHES]
    phases = [[(m, i) for i in range(lo, hi) for m in (1, 2)] for lo, hi in zip(bounds, bounds[1:])]
    batches = [[pair_copy(m, i) for m, i in ph] for ph in phases]
    batches[-1] += [pair_copy(0, i) for i in range(n_pairs)] + early_copies
    batches += [[wo_copy], [x_copy] + ffn_copies]

    def split_pair(m, i, after=None):
        low, high = np.uint32(0xFFFF), np.uint32(0xFFFF0000)
        if after is not None:
            zero = (pltpu.bitcast(after[:1], U32) >> 31) >> 1
            low, high = zero | low, zero | high
        even = stage_ref[m, i, pl.ds(0, d_model // 2, stride=2), :]
        odd = stage_ref[m, i, pl.ds(1, d_model // 2, stride=2), :]
        w_ref[m, 2 * i] = (even & low) | (odd << 16)
        w_ref[m, 2 * i + 1] = (even >> 16) | (odd & high)

    state = kv_ref.at[2 * n_heads + _ROT]
    first_at, second_at = pl.ds(n_tiles * seg, 8), pl.ds(n_tiles * seg + 8, 8)

    def stage_segment(s):
        xn = _layernorm(x_ref[s].astype(F32))
        for j in range(n_tiles):
            state[pl.ds(j * seg, seg), :] = xn[:, j * _LANES:(j + 1) * _LANES]

    for c in xpre_copies:
        c.start()
    for n, c in enumerate(xpre_copies):
        c.wait()
        for nxt in batches[n]:
            nxt.start()
        xpre = xpre_ref[pl.ds(n * half, half)].astype(F32).reshape(half * _PRE, d_model)
        xpre = _layernorm(xpre)
        lhs32_ref[pl.ds(n * half * _PRE, half * _PRE), :] = xpre
        lhs_ref[pl.ds(n * half * _PRE // 2, half * _PRE // 2), :] = pltpu.bitcast(xpre.astype(BF16), U32)
    for n, phase in enumerate(phases):
        for c in batches[n]:
            c.wait()
        for c in batches[n + 2]:
            c.start()
        for u, (m, i) in enumerate(phase):
            split_pair(m, i)
            for j in range(2):
                lhs = pltpu.bitcast(lhs_ref[...], BF16)
                y = _mm(lhs, pltpu.bitcast(w_ref[m, 2 * i + j], BF16))
                kv_ref[slot_of[m] + 2 * i + j] = y
                if phase is phases[-1]:
                    for iq in range(2 * u + j, n_pairs, 2 * len(phase)):
                        split_pair(0, iq, after=y)
    for t in range(1, _ROT):
        rows = pl.ds(0, t * _PRE)
        kv_ref[slot_of[0] + t, rows, :] = _mm(lhs32_ref[rows, :], pltpu.bitcast(w_ref[0, t], BF16))
    stage_segment(0)
    attn_ref[...] = jnp.zeros((seg, d_model), F32)
    state[first_at, :] = state[second_at, :] = jnp.zeros((8, _LANES), F32)
    wo_copy.wait()

    row = lax.broadcasted_iota(jnp.int32, (n_rows, n_rows), 0)
    col = lax.broadcasted_iota(jnp.int32, (n_rows, n_rows), 1)
    visible = (row >= seg) | (col >= seg) | (row >= col)
    seg_token = lax.broadcasted_iota(jnp.int32, (seg, _LANES), 0)
    token_bits = (n_seg * seg - 1).bit_length()
    token_mask = (1 << token_bits) - 1
    w_route = wr_ref[...].astype(F32)
    order = _issue_order(n_heads, cost_a=n_rows + 2 * (n_rows - _PRE))
    at = order.index(("A", 4))
    order[at:at] = [("F", 0), ("N", 0)]

    def routing_key(hn, s):
        prod = hn[:, :_LANES] * w_route[0:1]
        for j in range(1, n_tiles):
            prod = prod + hn[:, j * _LANES:(j + 1) * _LANES] * w_route[j:j + 1]
        r = jnp.broadcast_to(_rnd(jnp.sum(prod, axis=-1, keepdims=True)), (seg, _LANES))
        bits = pltpu.bitcast(r, jnp.int32) >> 16
        rank = jnp.where(bits < 0, ~bits, bits + 0x8000)
        rank = jnp.where(r == 0.0, 0x8000, jnp.where(r == r, rank, 0))
        key = _KEY_BASE + (rank << token_bits) + (token_mask - s * seg - seg_token)
        return pltpu.bitcast(key, F32)

    def finish_segment(s, live=True):
        h = _rnd(x_ref[s].astype(F32) + _rnd(attn_ref[...]))
        hn = _layernorm_rounded(h)
        h_ref[s] = h
        hn_ref[s] = hn
        out_ref[s] = (h + hn).astype(BF16)
        key = jnp.where(live, routing_key(hn, s), 0.0)
        first, second = state[first_at, :], state[second_at, :]
        for j in range(0, seg, 8):
            second = jnp.maximum(second, jnp.minimum(first, key[j:j + 8]))
            first = jnp.maximum(first, key[j:j + 8])
        state[first_at, :], state[second_at, :] = first, second

    def attend(s, turn, mem):
        xn = jnp.concatenate([state[pl.ds(j * seg, seg), :] for j in range(n_tiles)], axis=1)
        own = seg - _PRE
        pre = pl.ds(pl.multiple_of(s * _PRE, _PRE), _PRE)
        heads = [(turn + t) % _ROT for t in range(_ROT)] + list(range(_ROT, n_heads))

        def project(m, t):
            w = pltpu.bitcast(w_ref[m, heads[t]], BF16)
            if m == 0 and t >= _ROT:
                return _mm(jnp.concatenate([xn, mem], axis=0), w)
            if m == 0 and t == 0:
                first = jnp.minimum(s, n_seg - _ROT)
                ahead = pl.ds(pl.multiple_of(first * _PRE, _PRE), _ROT * _PRE)
                y = _mm(jnp.concatenate([xn[:own], lhs32_ref[ahead, :], mem], axis=0), w)
                kv_ref[slot_of[m] + heads[t], ahead, :] = y[own:-n_mem]
            else:
                y = _mm(jnp.concatenate([xn[:own], mem], axis=0), w)
            return jnp.concatenate(
                [y[:own], kv_ref[slot_of[m] + heads[t], pre, :], y[-n_mem:]], axis=0)

        q, k, v, p, o = {}, {}, {}, {}, {}
        acc = [None] * n_tiles
        for kind, t in order:
            if kind == "A":
                q[t] = project(0, t)
                k[t] = project(1, t).astype(BF16)
                v[t] = project(2, t).astype(BF16)
            elif kind == "B":
                sc = jnp.where(visible, _mm_t(q[t], k[t]) * scale, -1e9)
                e = jnp.exp(sc - jnp.max(sc, axis=-1, keepdims=True))
                p[t] = e / jnp.sum(e, axis=-1, keepdims=True)
            elif kind == "C":
                y = _mm(p[t], v[t])
                o[t] = jnp.concatenate([y[seg:], y[:seg]], axis=0)
            elif kind == "F":
                finish_segment((s + n_seg - 1) % n_seg, live=s > 0)
            elif kind == "N":
                stage_segment(jnp.minimum(s + 1, n_seg - 1))
            else:
                for j in range(n_tiles):
                    w = pltpu.bitcast(wo_ref[heads[t], :, j * _LANES:(j + 1) * _LANES], BF16)
                    y = _mm(o[t], w)
                    acc[j] = y if acc[j] is None else acc[j] + y
        y = jnp.concatenate(acc, axis=1)
        attn_ref[...] = y[n_mem:]
        return _rnd(y[:n_mem])

    def seg_body(it, mem):
        @pl.when(it == 1)
        def _():
            x_copy.wait()

        @pl.when(it >= 2)
        def _():
            blk = pl.ds((it - 2) * _UNROLL, _UNROLL)
            pltpu.make_async_copy(out_ref.at[blk], out_hbm.at[blk], out_sem).start()

        for u in range(_UNROLL):
            s = it * _UNROLL + u
            mem = attend(s, s if _UNROLL % _ROT else u, mem)
        return mem

    n_iter = n_seg // _UNROLL
    lax.fori_loop(0, n_iter, seg_body, mem0_ref[...].astype(F32))
    for c in ffn_copies:
        c.wait()
    finish_segment(n_seg - 1)
    blk = pl.ds((n_iter - 2) * _UNROLL, 2 * _UNROLL)
    pltpu.make_async_copy(out_ref.at[blk], out_hbm.at[blk], out_sem).start()

    first, second = state[first_at, :], state[second_at, :]
    best = jnp.max(first, axis=0, keepdims=True)
    runner_up = jnp.max(jnp.where(first == best, second, first), axis=0, keepdims=True)
    upper = lax.broadcasted_iota(jnp.int32, (8, _LANES), 0) == 0
    keys = pltpu.bitcast(jnp.where(upper, best, runner_up), jnp.int32) - _KEY_BASE
    tokens = jnp.minimum(token_mask - (keys & token_mask), n_seg * seg - 1)
    rank = keys >> token_bits
    score = pltpu.bitcast(jnp.where(rank < 0x8000, ~rank, rank - 0x8000) << 16, F32)
    (s0, r0), (s1, r1) = [(tokens[n, 0] // seg, tokens[n, 0] % seg) for n in range(2)]

    def picked(ref):
        upper = lax.broadcasted_iota(jnp.int32, (8, d_model), 0) == 0
        return jnp.where(upper, ref[s0, pl.ds(r0, 1), :], ref[s1, pl.ds(r1, 1), :])

    h_sel, hn_sel = picked(h_ref), picked(hn_ref)
    gate = _rnd(_mm(hn_sel, pltpu.bitcast(wg_ref[...], BF16)))
    up = _rnd(_mm(hn_sel, pltpu.bitcast(wu_ref[...], BF16)))
    act = _rnd(_rnd(gate * jax.nn.sigmoid(gate)) * up)
    y = _rnd(_mm(act, pltpu.bitcast(wd_ref[...], BF16)))
    y = _rnd(y * jnp.concatenate([_rnd(jax.nn.sigmoid(score))] * n_tiles, axis=1))
    new_rows = h_sel + _rnd(hn_sel + y)

    pltpu.make_async_copy(out_ref, out_hbm, out_sem).wait()
    seg_row = lax.broadcasted_iota(jnp.int32, (seg, d_model), 0)
    for n, (s, r) in enumerate(((s0, r0), (s1, r1))):
        old = out_ref[s].astype(F32)
        out_ref[s] = jnp.where(seg_row == r, new_rows[n:n + 1], old).astype(BF16)
    fix0 = pltpu.make_async_copy(out_ref.at[s0], out_hbm.at[s0], sem.at[11])
    fix1 = pltpu.make_async_copy(out_ref.at[s1], out_hbm.at[s1], sem.at[12])
    fix0.start()

    @pl.when(s0 != s1)
    def _():
        fix1.start()
        fix1.wait()

    fix0.wait()


@functools.partial(jax.jit, static_argnames=("A_seg_len",))
def pallas_sequential_preLN__memory_aug_recurrent_mem_tr__moe_arch_mod__prompt_kernel(
    A_x: jax.Array,
    A_mem0: jax.Array,
    A_Wq: jax.Array,
    A_Wk: jax.Array,
    A_Wv: jax.Array,
    A_Wo: jax.Array,
    A_seg_len: int,
    B_x: jax.Array,
    B_w_r: jax.Array,
    B_w_gate: jax.Array,
    B_w_up: jax.Array,
    B_w_down: jax.Array,
):
    del B_x
    batch, seq, d_model = A_x.shape
    n_mem = A_mem0.shape[1]
    _, n_heads, d_head = A_Wq.shape
    d_ff = B_w_gate.shape[1]
    seg = int(A_seg_len)
    n_seg = seq // seg
    assert batch == 1 and seq == n_seg * seg and seq <= 1 << 13 and n_seg % _UNROLL == 0

    hbm = pl.BlockSpec(memory_space=pl.ANY)
    out = pl.pallas_call(
        _kernel,
        out_shape=jax.ShapeDtypeStruct((n_seg, seg, d_model), A_x.dtype),
        in_specs=[hbm] * 10,
        out_specs=hbm,
        scratch_shapes=[
            pltpu.VMEM((n_mem, d_model), BF16),
            pltpu.VMEM((d_model // _LANES, _LANES), BF16),
            pltpu.VMEM((n_seg, seg, d_model), BF16),
            pltpu.VMEM((n_seg, _PRE, d_model), BF16),
            pltpu.VMEM((n_seg * _PRE // 2, d_model), U32),
            pltpu.VMEM((n_seg * _PRE, d_model), F32),
            pltpu.VMEM((3, n_heads // 2, d_model, d_head), U32),
            pltpu.VMEM((3, n_heads, d_model // 2, d_head), U32),
            pltpu.VMEM((n_heads, d_head // 2, d_model), U32),
            pltpu.VMEM((d_model // 2, d_ff), U32),
            pltpu.VMEM((d_model // 2, d_ff), U32),
            pltpu.VMEM((d_ff // 2, d_model), U32),
            pltpu.VMEM((2 * n_heads + _ROT + 1, n_seg * _PRE, d_head), F32),
            pltpu.VMEM((seg, d_model), F32),
            pltpu.VMEM((n_seg, seg, d_model), F32),
            pltpu.VMEM((n_seg, seg, d_model), F32),
            pltpu.VMEM((n_seg, seg, d_model), BF16),
            pltpu.SemaphoreType.DMA((3 * n_heads // 2,)),
            pltpu.SemaphoreType.DMA((13,)),
        ],
        compiler_params=pltpu.CompilerParams(vmem_limit_bytes=100 * 1024 * 1024),
        name="rmt_mod",
    )(
        A_x.reshape(n_seg, seg, d_model),
        A_mem0.reshape(n_mem, d_model),
        A_Wq, A_Wk, A_Wv, A_Wo,
        B_w_r.reshape(d_model // _LANES, _LANES),
        B_w_gate, B_w_up, B_w_down,
    )
    return out.reshape(batch, seq, d_model)
```

```python
import functools

import jax
import jax.numpy as jnp
import numpy as np
from jax import lax
import jax.experimental.pallas as pl
import jax.experimental.pallas.tpu as pltpu

F32 = jnp.float32
BF16 = jnp.bfloat16
U32 = jnp.uint32

_LANES = 128
_EPS = 1e-5
_PRE = 8
_KEY_BASE = 1 << 29
_UNROLL = 4
_Q_HEADS = 2 * _UNROLL
_PHASES = (0, 1, 3, 7, 15, 24, 32)


def _mm(a, b):
    return lax.dot_general(a, b, (((1,), (0,)), ((), ())), preferred_element_type=F32)


def _mm_t(a, b):
    return lax.dot_general(a, b, (((1,), (1,)), ((), ())), preferred_element_type=F32)


def _rnd(x):
    return x.astype(BF16).astype(F32)


def _moments(x):
    inv_n = 1.0 / x.shape[-1]
    mean = jnp.sum(x, axis=-1, keepdims=True) * inv_n
    c = x - mean
    return mean, c, jnp.sum(c * c, axis=-1, keepdims=True) * inv_n


def _layernorm(x):
    _, c, var = _moments(x)
    return c * lax.rsqrt(var + _EPS)


def _layernorm_rounded(x):
    mean, _, var = _moments(x)
    den = _rnd(jnp.sqrt(_rnd(_rnd(var) + float(np.asarray(_EPS, dtype=BF16)))))
    return _rnd(_rnd(x - _rnd(mean)) / den)


def _issue_order(n_heads, cost_a, lat_ab=200, lat_bc=480, lat_cd=200, defer=28, group=2):
    cost = dict(A=cost_a, B=10, C=10, D=40)
    width = dict(A=1, B=group, C=group, D=1)
    wait = dict(B=("A", lat_ab), C=("B", lat_bc), D=("C", lat_cd))
    nxt = dict.fromkeys(cost, 0)
    ops, done, t = [], {}, 0

    def ready(kind):
        src, lat = wait[kind]
        last = nxt[kind] + width[kind] - 1
        return last < nxt[src] and t >= done[src, last] + lat

    while nxt["D"] < n_heads:
        kind = next((c for c in "CB" if ready(c)), None)
        if kind is None and ready("D") and (nxt["A"] == n_heads or nxt["A"] - nxt["D"] > defer):
            kind = "D"
        if kind is None and nxt["A"] < n_heads:
            kind = "A"
        if kind is None:
            t += 10
            continue
        for _ in range(width[kind]):
            t += cost[kind]
            ops.append((kind, nxt[kind]))
            done[kind, nxt[kind]] = t
            nxt[kind] += 1
    return ops


def _kernel(
    x_hbm, mem0_hbm, wq_hbm, wk_hbm, wv_hbm, wo_hbm, wr_hbm, wg_hbm, wu_hbm, wd_hbm,
    out_hbm,
    mem0_ref, wr_ref, x_ref, xpre_ref, lhs_ref, lhs32_ref, stage_ref, w_ref, wo_ref, wg_ref, wu_ref, wd_ref,
    kv_ref, attn_ref, h_ref, hn_ref, out_ref, sem,
):
    n_seg, seg, d_model = x_hbm.shape
    n_mem = mem0_ref.shape[0]
    n_heads, d_head = wo_hbm.shape[0], wo_hbm.shape[1]
    n_pairs = n_heads // 2
    n_tiles = d_model // _LANES
    n_rows = seg + n_mem
    scale = float(np.asarray(d_head ** -0.5, dtype=BF16))

    w_words = [w.bitcast(U32) for w in (wq_hbm, wk_hbm, wv_hbm)]

    slot_of = (2 * n_heads, 0, n_heads)
    half = n_seg // 2
    x_head, x_rest = pl.ds(0, _UNROLL + 1), pl.ds(_UNROLL + 1, n_seg - _UNROLL - 1)

    def pair(m, i):
        return w_words[m].at[:, i, :], stage_ref.at[m, i]

    units = [(m, i) for i in range(n_pairs) for m in (1, 2)]
    bounds = [len(units) * n // _PHASES[-1] for n in _PHASES]
    phases = [units[lo:hi] for lo, hi in zip(bounds, bounds[1:])]
    batches = [
        [(x_hbm.at[pl.ds(n * half, half), pl.ds(seg - _PRE, _PRE), :], xpre_ref.at[pl.ds(n * half, half)])]
        for n in range(2)
    ]
    batches += [[pair(m, i) for m, i in phase] for phase in phases]
    batches[-1] += [pair(0, i) for i in range(n_pairs)]
    batches[-1] += [(x_hbm.at[x_head], x_ref.at[x_head]), (mem0_hbm, mem0_ref), (wr_hbm, wr_ref)]
    batches.append([(wo_hbm.bitcast(U32), wo_ref)])
    batches.append([
        (x_hbm.at[x_rest], x_ref.at[x_rest]),
        (wg_hbm.bitcast(U32), wg_ref), (wu_hbm.bitcast(U32), wu_ref), (wd_hbm.bitcast(U32), wd_ref),
    ])
    out_sem = sem.at[len(batches)]

    def start(n):
        for src, dst in batches[n]:
            pltpu.make_async_copy(src, dst, sem.at[n]).start()

    def wait(n):
        for src, dst in batches[n]:
            pltpu.make_async_copy(src, dst, sem.at[n]).wait()

    def split_pair(m, i, after=None):
        rows = d_model // 2 // n_tiles
        for c in range(n_tiles):
            low, high = np.uint32(0xFFFF), np.uint32(0xFFFF0000)
            if after is not None:
                at = after.shape[0] // n_tiles * c
                zero = (pltpu.bitcast(after[at:at + 1], U32) >> 31) >> 1
                low, high = zero | low, zero | high
            even = stage_ref[m, i, pl.ds(2 * c * rows, rows, stride=2), :]
            odd = stage_ref[m, i, pl.ds(2 * c * rows + 1, rows, stride=2), :]
            w_ref[m, 2 * i, pl.ds(c * rows, rows), :] = (even & low) | (odd << 16)
            w_ref[m, 2 * i + 1, pl.ds(c * rows, rows), :] = (even >> 16) | (odd & high)

    state = kv_ref.at[2 * n_heads + _Q_HEADS]
    first_at, second_at = pl.ds(n_tiles * seg, 8), pl.ds(n_tiles * seg + 8, 8)

    def stage_segment(s):
        xn = _layernorm(x_ref[s].astype(F32))
        for j in range(n_tiles):
            state[pl.ds(j * seg, seg), :] = xn[:, j * _LANES:(j + 1) * _LANES]

    start(0)
    start(1)
    for n in range(2):
        wait(n)
        start(n + 2)
        xpre = xpre_ref[pl.ds(n * half, half)].astype(F32).reshape(half * _PRE, d_model)
        xpre = _layernorm(xpre)
        lhs32_ref[pl.ds(n * half * _PRE, half * _PRE), :] = xpre
        lhs_ref[pl.ds(n * half * _PRE // 2, half * _PRE // 2), :] = pltpu.bitcast(xpre.astype(BF16), U32)
    for n, phase in enumerate(phases):
        wait(n + 2)
        start(n + 4)
        for u, (m, i) in enumerate(phase):
            split_pair(m, i)
            for j in range(2):
                lhs = pltpu.bitcast(lhs_ref[...], BF16)
                y = _mm(lhs, pltpu.bitcast(w_ref[m, 2 * i + j], BF16))
                kv_ref[slot_of[m] + 2 * i + j] = y
                if phase is phases[-1]:
                    for iq in range(2 * u + j, n_pairs, 2 * len(phase)):
                        split_pair(0, iq, after=y)
    for t in range(_Q_HEADS):
        if t % _UNROLL:
            rows = pl.ds(0, t % _UNROLL * _PRE)
            kv_ref[slot_of[0] + t, rows, :] = _mm(lhs32_ref[rows, :], pltpu.bitcast(w_ref[0, t], BF16))
    stage_segment(0)
    attn_ref[...] = jnp.zeros((seg, d_model), F32)
    state[first_at, :] = state[second_at, :] = jnp.zeros((8, _LANES), F32)
    wait(len(batches) - 2)

    row = lax.broadcasted_iota(jnp.int32, (n_rows, n_rows), 0)
    col = lax.broadcasted_iota(jnp.int32, (n_rows, n_rows), 1)
    visible = (row >= seg) | (col >= seg) | (row >= col)
    seg_token = lax.broadcasted_iota(jnp.int32, (seg, _LANES), 0)
    token_bits = (n_seg * seg - 1).bit_length()
    token_mask = (1 << token_bits) - 1
    w_route = wr_ref[...].astype(F32)
    order = _issue_order(n_heads, cost_a=n_rows + 2 * (n_rows - _PRE))
    at = order.index(("A", 4))
    order[at:at] = [("F", 0), ("N", 0)]

    def routing_key(hn, s):
        prod = hn[:, :_LANES] * w_route[0:1]
        for j in range(1, n_tiles):
            prod = prod + hn[:, j * _LANES:(j + 1) * _LANES] * w_route[j:j + 1]
        r = jnp.broadcast_to(_rnd(jnp.sum(prod, axis=-1, keepdims=True)), (seg, _LANES))
        bits = pltpu.bitcast(r, jnp.int32) >> 16
        rank = jnp.where(bits < 0, ~bits, bits + 0x8000)
        rank = jnp.where(r == 0.0, 0x8000, jnp.where(r == r, rank, 0))
        key = _KEY_BASE + (rank << token_bits) + (token_mask - s * seg - seg_token)
        return pltpu.bitcast(key, F32)

    def finish_segment(s, live=True):
        h = _rnd(x_ref[s].astype(F32) + _rnd(attn_ref[...]))
        hn = _layernorm_rounded(h)
        h_ref[s] = h
        hn_ref[s] = hn
        out_ref[s] = (h + hn).astype(BF16)
        key = jnp.where(live, routing_key(hn, s), 0.0)
        first, second = state[first_at, :], state[second_at, :]
        for j in range(0, seg, 8):
            second = jnp.maximum(second, jnp.minimum(first, key[j:j + 8]))
            first = jnp.maximum(first, key[j:j + 8])
        state[first_at, :], state[second_at, :] = first, second

    def attend(s, turn, mem):
        xn = jnp.concatenate([state[pl.ds(j * seg, seg), :] for j in range(n_tiles)], axis=1)
        own = seg - _PRE
        pre = pl.ds(pl.multiple_of(s * _PRE, _PRE), _PRE)
        heads = [(turn + t) % _UNROLL for t in range(_UNROLL)] + list(range(_UNROLL, n_heads))

        first = jnp.minimum(s, n_seg - _UNROLL)
        ahead = pl.ds(pl.multiple_of(first * _PRE, _PRE), _UNROLL * _PRE)
        for t in range(_UNROLL + turn, _Q_HEADS, _UNROLL):
            kv_ref[slot_of[0] + t, ahead, :] = _mm(lhs32_ref[ahead, :], pltpu.bitcast(w_ref[0, t], BF16))

        def project(m, t):
            w = pltpu.bitcast(w_ref[m, heads[t]], BF16)
            if m == 0 and t >= _Q_HEADS:
                return _mm(jnp.concatenate([xn, mem], axis=0), w)
            if m == 0 and t == 0:
                y = _mm(jnp.concatenate([xn[:own], lhs32_ref[ahead, :], mem], axis=0), w)
                kv_ref[slot_of[m] + heads[t], ahead, :] = y[own:-n_mem]
            else:
                y = _mm(jnp.concatenate([xn[:own], mem], axis=0), w)
            return jnp.concatenate(
                [y[:own], kv_ref[slot_of[m] + heads[t], pre, :], y[-n_mem:]], axis=0)

        q, k, v, p, o = {}, {}, {}, {}, {}
        acc = [None] * n_tiles
        for kind, t in order:
            if kind == "A":
                q[t] = project(0, t)
                k[t] = project(1, t).astype(BF16)
                v[t] = project(2, t).astype(BF16)
            elif kind == "B":
                sc = jnp.where(visible, _mm_t(q[t], k[t]) * scale, -1e9)
                e = jnp.exp(sc - jnp.max(sc, axis=-1, keepdims=True))
                p[t] = e / jnp.sum(e, axis=-1, keepdims=True)
            elif kind == "C":
                y = _mm(p[t], v[t])
                o[t] = jnp.concatenate([y[seg:], y[:seg]], axis=0)
            elif kind == "F":
                finish_segment((s + n_seg - 1) % n_seg, live=s > 0)
            elif kind == "N":
                stage_segment(jnp.minimum(s + 1, n_seg - 1))
            else:
                for j in range(n_tiles):
                    w = pltpu.bitcast(wo_ref[heads[t], :, j * _LANES:(j + 1) * _LANES], BF16)
                    y = _mm(o[t], w)
                    acc[j] = y if acc[j] is None else acc[j] + y
        y = jnp.concatenate(acc, axis=1)
        attn_ref[...] = y[n_mem:]
        return _rnd(y[:n_mem])

    def seg_body(it, mem):
        @pl.when(it == 1)
        def _():
            wait(len(batches) - 1)

        @pl.when(it >= 2)
        def _():
            blk = pl.ds((it - 2) * _UNROLL, _UNROLL)
            pltpu.make_async_copy(out_ref.at[blk], out_hbm.at[blk], out_sem).start()

        for u in range(_UNROLL):
            mem = attend(it * _UNROLL + u, u, mem)
        return mem

    n_iter = n_seg // _UNROLL
    lax.fori_loop(0, n_iter, seg_body, mem0_ref[...].astype(F32))
    finish_segment(n_seg - 1)
    blk = pl.ds((n_iter - 2) * _UNROLL, 2 * _UNROLL)
    pltpu.make_async_copy(out_ref.at[blk], out_hbm.at[blk], out_sem).start()

    first, second = state[first_at, :], state[second_at, :]
    best = jnp.max(first, axis=0, keepdims=True)
    runner_up = jnp.max(jnp.where(first == best, second, first), axis=0, keepdims=True)
    upper = lax.broadcasted_iota(jnp.int32, (8, _LANES), 0) == 0
    keys = pltpu.bitcast(jnp.where(upper, best, runner_up), jnp.int32) - _KEY_BASE
    tokens = jnp.minimum(token_mask - (keys & token_mask), n_seg * seg - 1)
    rank = keys >> token_bits
    score = pltpu.bitcast(jnp.where(rank < 0x8000, ~rank, rank - 0x8000) << 16, F32)
    (s0, r0), (s1, r1) = [(tokens[n, 0] // seg, tokens[n, 0] % seg) for n in range(2)]

    def picked(ref):
        upper = lax.broadcasted_iota(jnp.int32, (8, d_model), 0) == 0
        return jnp.where(upper, ref[s0, pl.ds(r0, 1), :], ref[s1, pl.ds(r1, 1), :])

    h_sel, hn_sel = picked(h_ref), picked(hn_ref)
    gate = _rnd(_mm(hn_sel, pltpu.bitcast(wg_ref[...], BF16)))
    up = _rnd(_mm(hn_sel, pltpu.bitcast(wu_ref[...], BF16)))
    act = _rnd(_rnd(gate * jax.nn.sigmoid(gate)) * up)
    y = _rnd(_mm(act, pltpu.bitcast(wd_ref[...], BF16)))
    y = _rnd(y * jnp.concatenate([_rnd(jax.nn.sigmoid(score))] * n_tiles, axis=1))
    new_rows = h_sel + _rnd(hn_sel + y)

    pltpu.make_async_copy(out_ref, out_hbm, out_sem).wait()
    seg_row = lax.broadcasted_iota(jnp.int32, (seg, d_model), 0)
    for n, (s, r) in enumerate(((s0, r0), (s1, r1))):
        old = out_ref[s].astype(F32)
        out_ref[s] = jnp.where(seg_row == r, new_rows[n:n + 1], old).astype(BF16)
    fix0 = pltpu.make_async_copy(out_ref.at[s0], out_hbm.at[s0], sem.at[0])
    fix1 = pltpu.make_async_copy(out_ref.at[s1], out_hbm.at[s1], sem.at[1])
    fix0.start()

    @pl.when(s0 != s1)
    def _():
        fix1.start()
        fix1.wait()

    fix0.wait()


@functools.partial(jax.jit, static_argnames=("A_seg_len",))
def pallas_sequential_preLN__memory_aug_recurrent_mem_tr__moe_arch_mod__prompt_kernel(
    A_x: jax.Array,
    A_mem0: jax.Array,
    A_Wq: jax.Array,
    A_Wk: jax.Array,
    A_Wv: jax.Array,
    A_Wo: jax.Array,
    A_seg_len: int,
    B_x: jax.Array,
    B_w_r: jax.Array,
    B_w_gate: jax.Array,
    B_w_up: jax.Array,
    B_w_down: jax.Array,
):
    del B_x
    batch, seq, d_model = A_x.shape
    n_mem = A_mem0.shape[1]
    _, n_heads, d_head = A_Wq.shape
    d_ff = B_w_gate.shape[1]
    seg = int(A_seg_len)
    n_seg = seq // seg
    assert batch == 1 and seq == n_seg * seg and seq <= 1 << 13 and n_seg % _UNROLL == 0

    hbm = pl.BlockSpec(memory_space=pl.ANY)
    out = pl.pallas_call(
        _kernel,
        out_shape=jax.ShapeDtypeStruct((n_seg, seg, d_model), A_x.dtype),
        in_specs=[hbm] * 10,
        out_specs=hbm,
        scratch_shapes=[
            pltpu.VMEM((n_mem, d_model), BF16),
            pltpu.VMEM((d_model // _LANES, _LANES), BF16),
            pltpu.VMEM((n_seg, seg, d_model), BF16),
            pltpu.VMEM((n_seg, _PRE, d_model), BF16),
            pltpu.VMEM((n_seg * _PRE // 2, d_model), U32),
            pltpu.VMEM((n_seg * _PRE, d_model), F32),
            pltpu.VMEM((3, n_heads // 2, d_model, d_head), U32),
            pltpu.VMEM((3, n_heads, d_model // 2, d_head), U32),
            pltpu.VMEM((n_heads, d_head // 2, d_model), U32),
            pltpu.VMEM((d_model // 2, d_ff), U32),
            pltpu.VMEM((d_model // 2, d_ff), U32),
            pltpu.VMEM((d_ff // 2, d_model), U32),
            pltpu.VMEM((2 * n_heads + _Q_HEADS + 1, n_seg * _PRE, d_head), F32),
            pltpu.VMEM((seg, d_model), F32),
            pltpu.VMEM((n_seg, seg, d_model), F32),
            pltpu.VMEM((n_seg, seg, d_model), F32),
            pltpu.VMEM((n_seg, seg, d_model), BF16),
            pltpu.SemaphoreType.DMA((len(_PHASES) + 4,)),
        ],
        compiler_params=pltpu.CompilerParams(vmem_limit_bytes=100 * 1024 * 1024),
        name="rmt_mod",
    )(
        A_x.reshape(n_seg, seg, d_model),
        A_mem0.reshape(n_mem, d_model),
        A_Wq, A_Wk, A_Wv, A_Wo,
        B_w_r.reshape(d_model // _LANES, _LANES),
        B_w_gate, B_w_up, B_w_down,
    )
    return out.reshape(batch, seq, d_model)
```

```python
import functools

import jax
import jax.numpy as jnp
import numpy as np
from jax import lax
import jax.experimental.pallas as pl
import jax.experimental.pallas.tpu as pltpu

F32 = jnp.float32
BF16 = jnp.bfloat16
U32 = jnp.uint32

_LANES = 128
_EPS = 1e-5
_PRE = 8
_KEY_BASE = 1 << 29
_UNROLL = 4
_Q_HEADS = 2 * _UNROLL
_PHASES = (0, 1, 3, 7, 15, 24, 32)


def _mm(a, b):
    return lax.dot_general(a, b, (((1,), (0,)), ((), ())), preferred_element_type=F32)


def _mm_t(a, b):
    return lax.dot_general(a, b, (((1,), (1,)), ((), ())), preferred_element_type=F32)


def _rnd(x):
    return x.astype(BF16).astype(F32)


def _moments(x):
    inv_n = 1.0 / x.shape[-1]
    mean = jnp.sum(x, axis=-1, keepdims=True) * inv_n
    c = x - mean
    return mean, c, jnp.sum(c * c, axis=-1, keepdims=True) * inv_n


def _layernorm(x):
    _, c, var = _moments(x)
    return c * lax.rsqrt(var + _EPS)


def _layernorm_rounded(x):
    mean, _, var = _moments(x)
    den = _rnd(jnp.sqrt(_rnd(_rnd(var) + float(np.asarray(_EPS, dtype=BF16)))))
    return _rnd(_rnd(x - _rnd(mean)) / den)


def _issue_order(n_heads, cost_a, lat_ab=200, lat_bc=480, lat_cd=200, defer=28, group=2):
    cost = dict(A=cost_a, B=10, C=10, D=40)
    width = dict(A=1, B=group, C=group, D=1)
    wait = dict(B=("A", lat_ab), C=("B", lat_bc), D=("C", lat_cd))
    nxt = dict.fromkeys(cost, 0)
    ops, done, t = [], {}, 0

    def ready(kind):
        src, lat = wait[kind]
        last = nxt[kind] + width[kind] - 1
        return last < nxt[src] and t >= done[src, last] + lat

    while nxt["D"] < n_heads:
        kind = next((c for c in "CB" if ready(c)), None)
        if kind is None and ready("D") and (nxt["A"] == n_heads or nxt["A"] - nxt["D"] > defer):
            kind = "D"
        if kind is None and nxt["A"] < n_heads:
            kind = "A"
        if kind is None:
            t += 10
            continue
        for _ in range(width[kind]):
            t += cost[kind]
            ops.append((kind, nxt[kind]))
            done[kind, nxt[kind]] = t
            nxt[kind] += 1
    return ops


def _kernel(
    x_hbm, mem0_hbm, wq_hbm, wk_hbm, wv_hbm, wo_hbm, wr_hbm, wg_hbm, wu_hbm, wd_hbm,
    out_hbm,
    mem0_ref, wr_ref, x_ref, xpre_ref, lhs_ref, lhs32_ref, stage_ref, w_ref, wo_ref, wg_ref, wu_ref, wd_ref,
    kv_ref, attn_ref, h_ref, hn_ref, out_ref, sem,
):
    n_seg, seg, d_model = x_hbm.shape
    n_mem = mem0_ref.shape[0]
    n_heads, d_head = wo_hbm.shape[0], wo_hbm.shape[1]
    n_pairs = n_heads // 2
    n_tiles = d_model // _LANES
    n_rows = seg + n_mem
    scale = float(np.asarray(d_head ** -0.5, dtype=BF16))

    w_words = [w.bitcast(U32) for w in (wq_hbm, wk_hbm, wv_hbm)]

    slot_of = (2 * n_heads, 0, n_heads)
    half = n_seg // 2
    x_head, x_rest = pl.ds(0, _UNROLL + 1), pl.ds(_UNROLL + 1, n_seg - _UNROLL - 1)

    def pair(m, i):
        return w_words[m].at[:, i, :], stage_ref.at[m, i]

    units = [(m, i) for i in range(n_pairs) for m in (1, 2)]
    bounds = [len(units) * n // _PHASES[-1] for n in _PHASES]
    phases = [units[lo:hi] for lo, hi in zip(bounds, bounds[1:])]
    batches = [
        [(x_hbm.at[pl.ds(n * half, half), pl.ds(seg - _PRE, _PRE), :], xpre_ref.at[pl.ds(n * half, half)])]
        for n in range(2)
    ]
    batches += [[pair(m, i) for m, i in phase] for phase in phases]
    batches[-1] += [pair(0, i) for i in range(n_pairs)]
    batches[-1] += [(x_hbm.at[x_head], x_ref.at[x_head]), (mem0_hbm, mem0_ref), (wr_hbm, wr_ref)]
    batches.append([(wo_hbm.bitcast(U32), wo_ref)])
    batches.append([
        (x_hbm.at[x_rest], x_ref.at[x_rest]),
        (wg_hbm.bitcast(U32), wg_ref), (wu_hbm.bitcast(U32), wu_ref), (wd_hbm.bitcast(U32), wd_ref),
    ])
    out_sem = sem.at[len(batches)]

    def start(n):
        for src, dst in batches[n]:
            pltpu.make_async_copy(src, dst, sem.at[n]).start()

    def wait(n):
        for src, dst in batches[n]:
            pltpu.make_async_copy(src, dst, sem.at[n]).wait()

    def split_pair(m, i, after=None):
        for c in range(n_tiles):
            shift, high = np.uint32(16), np.uint32(0xFFFF0000)
            if after is not None:
                at = after.shape[0] // n_tiles * c
                zero = (pltpu.bitcast(after[at:at + 1], U32) >> 31) >> 1
                shift, high = zero | shift, zero | high
            words = stage_ref[m, i, pl.ds(c * _LANES, _LANES), :]
            for j, bits in enumerate((words << shift, words & high)):
                w_ref[m, 2 * i + j, pl.ds(c * _LANES // 2, _LANES // 2), :] = pltpu.bitcast(
                    pltpu.bitcast(bits, F32).astype(BF16), U32)

    state = kv_ref.at[2 * n_heads + _Q_HEADS]
    first_at, second_at = pl.ds(n_tiles * seg, 8), pl.ds(n_tiles * seg + 8, 8)

    def stage_segment(s):
        xn = _layernorm(x_ref[s].astype(F32))
        for j in range(n_tiles):
            state[pl.ds(j * seg, seg), :] = xn[:, j * _LANES:(j + 1) * _LANES]

    start(0)
    start(1)
    for n in range(2):
        wait(n)
        start(n + 2)
        xpre = xpre_ref[pl.ds(n * half, half)].astype(F32).reshape(half * _PRE, d_model)
        xpre = _layernorm(xpre)
        lhs32_ref[pl.ds(n * half * _PRE, half * _PRE), :] = xpre
        lhs_ref[pl.ds(n * half * _PRE // 2, half * _PRE // 2), :] = pltpu.bitcast(xpre.astype(BF16), U32)
    for n, phase in enumerate(phases):
        wait(n + 2)
        start(n + 4)
        for u, (m, i) in enumerate(phase):
            split_pair(m, i)
            for j in range(2):
                lhs = pltpu.bitcast(lhs_ref[...], BF16)
                y = _mm(lhs, pltpu.bitcast(w_ref[m, 2 * i + j], BF16))
                kv_ref[slot_of[m] + 2 * i + j] = y
                if phase is phases[-1]:
                    for iq in range(2 * u + j, n_pairs, 2 * len(phase)):
                        split_pair(0, iq, after=y)
    for t in range(_Q_HEADS):
        if t % _UNROLL:
            rows = pl.ds(0, t % _UNROLL * _PRE)
            kv_ref[slot_of[0] + t, rows, :] = _mm(lhs32_ref[rows, :], pltpu.bitcast(w_ref[0, t], BF16))
    stage_segment(0)
    attn_ref[...] = jnp.zeros((seg, d_model), F32)
    state[first_at, :] = state[second_at, :] = jnp.zeros((8, _LANES), F32)
    wait(len(batches) - 2)

    row = lax.broadcasted_iota(jnp.int32, (n_rows, n_rows), 0)
    col = lax.broadcasted_iota(jnp.int32, (n_rows, n_rows), 1)
    visible = (row >= seg) | (col >= seg) | (row >= col)
    seg_token = lax.broadcasted_iota(jnp.int32, (seg, _LANES), 0)
    token_bits = (n_seg * seg - 1).bit_length()
    token_mask = (1 << token_bits) - 1
    w_route = wr_ref[...].astype(F32)
    order = _issue_order(n_heads, cost_a=n_rows + 2 * (n_rows - _PRE))
    at = order.index(("A", 4))
    order[at:at] = [("F", 0), ("N", 0)]

    def routing_key(hn, s):
        prod = hn[:, :_LANES] * w_route[0:1]
        for j in range(1, n_tiles):
            prod = prod + hn[:, j * _LANES:(j + 1) * _LANES] * w_route[j:j + 1]
        r = jnp.broadcast_to(_rnd(jnp.sum(prod, axis=-1, keepdims=True)), (seg, _LANES))
        bits = pltpu.bitcast(r, jnp.int32) >> 16
        rank = jnp.where(bits < 0, ~bits, bits + 0x8000)
        rank = jnp.where(r == 0.0, 0x8000, jnp.where(r == r, rank, 0))
        key = _KEY_BASE + (rank << token_bits) + (token_mask - s * seg - seg_token)
        return pltpu.bitcast(key, F32)

    def finish_segment(s, live=True):
        h = _rnd(x_ref[s].astype(F32) + _rnd(attn_ref[...]))
        hn = _layernorm_rounded(h)
        h_ref[s] = h
        hn_ref[s] = hn
        out_ref[s] = (h + hn).astype(BF16)
        key = jnp.where(live, routing_key(hn, s), 0.0)
        first, second = state[first_at, :], state[second_at, :]
        for j in range(0, seg, 8):
            second = jnp.maximum(second, jnp.minimum(first, key[j:j + 8]))
            first = jnp.maximum(first, key[j:j + 8])
        state[first_at, :], state[second_at, :] = first, second

    def attend(s, turn, mem):
        xn = jnp.concatenate([state[pl.ds(j * seg, seg), :] for j in range(n_tiles)], axis=1)
        own = seg - _PRE
        pre = pl.ds(pl.multiple_of(s * _PRE, _PRE), _PRE)
        heads = [(turn + t) % _UNROLL for t in range(_UNROLL)] + list(range(_UNROLL, n_heads))

        first = jnp.minimum(s, n_seg - _UNROLL)
        ahead = pl.ds(pl.multiple_of(first * _PRE, _PRE), _UNROLL * _PRE)
        for t in range(_UNROLL + turn, _Q_HEADS, _UNROLL):
            kv_ref[slot_of[0] + t, ahead, :] = _mm(lhs32_ref[ahead, :], pltpu.bitcast(w_ref[0, t], BF16))

        def project(m, t):
            w = pltpu.bitcast(w_ref[m, heads[t]], BF16)
            if m == 0 and t >= _Q_HEADS:
                return _mm(jnp.concatenate([xn, mem], axis=0), w)
            if m == 0 and t == 0:
                y = _mm(jnp.concatenate([xn[:own], lhs32_ref[ahead, :], mem], axis=0), w)
                kv_ref[slot_of[m] + heads[t], ahead, :] = y[own:-n_mem]
            else:
                y = _mm(jnp.concatenate([xn[:own], mem], axis=0), w)
            return jnp.concatenate(
                [y[:own], kv_ref[slot_of[m] + heads[t], pre, :], y[-n_mem:]], axis=0)

        q, k, v, p, o = {}, {}, {}, {}, {}
        acc = [None] * n_tiles
        for kind, t in order:
            if kind == "A":
                q[t] = project(0, t)
                k[t] = project(1, t).astype(BF16)
                v[t] = project(2, t).astype(BF16)
            elif kind == "B":
                sc = jnp.where(visible, _mm_t(q[t], k[t]) * scale, -1e9)
                e = jnp.exp(sc - jnp.max(sc, axis=-1, keepdims=True))
                p[t] = e / jnp.sum(e, axis=-1, keepdims=True)
            elif kind == "C":
                y = _mm(p[t], v[t])
                o[t] = jnp.concatenate([y[seg:], y[:seg]], axis=0)
            elif kind == "F":
                finish_segment(jnp.maximum(s - 1, 0), live=s > 0)
            elif kind == "N":
                stage_segment(jnp.minimum(s + 1, n_seg - 1))
            else:
                for j in range(n_tiles):
                    w = pltpu.bitcast(wo_ref[heads[t], :, j * _LANES:(j + 1) * _LANES], BF16)
                    y = _mm(o[t], w)
                    acc[j] = y if acc[j] is None else acc[j] + y
        y = jnp.concatenate(acc, axis=1)
        attn_ref[...] = y[n_mem:]
        return _rnd(y[:n_mem])

    def seg_body(it, mem):
        @pl.when(it == 1)
        def _():
            wait(len(batches) - 1)

        @pl.when(it == n_iter - 1)
        def _():
            blk = pl.ds(0, n_seg - _UNROLL - 1)
            pltpu.make_async_copy(out_ref.at[blk], out_hbm.at[blk], out_sem).start()

        for u in range(_UNROLL):
            mem = attend(it * _UNROLL + u, u, mem)
        return mem

    n_iter = n_seg // _UNROLL
    lax.fori_loop(0, n_iter, seg_body, mem0_ref[...].astype(F32))
    finish_segment(n_seg - 1)
    blk = pl.ds(n_seg - _UNROLL - 1, _UNROLL + 1)
    pltpu.make_async_copy(out_ref.at[blk], out_hbm.at[blk], out_sem).start()

    first, second = state[first_at, :], state[second_at, :]
    best = jnp.max(first, axis=0, keepdims=True)
    runner_up = jnp.max(jnp.where(first == best, second, first), axis=0, keepdims=True)
    upper = lax.broadcasted_iota(jnp.int32, (8, _LANES), 0) == 0
    keys = pltpu.bitcast(jnp.where(upper, best, runner_up), jnp.int32) - _KEY_BASE
    tokens = jnp.minimum(token_mask - (keys & token_mask), n_seg * seg - 1)
    rank = keys >> token_bits
    score = pltpu.bitcast(jnp.where(rank < 0x8000, ~rank, rank - 0x8000) << 16, F32)
    (s0, r0), (s1, r1) = [(tokens[n, 0] // seg, tokens[n, 0] % seg) for n in range(2)]

    def picked(ref):
        upper = lax.broadcasted_iota(jnp.int32, (8, d_model), 0) == 0
        return jnp.where(upper, ref[s0, pl.ds(r0, 1), :], ref[s1, pl.ds(r1, 1), :])

    h_sel, hn_sel = picked(h_ref), picked(hn_ref)
    gate = _rnd(_mm(hn_sel, pltpu.bitcast(wg_ref[...], BF16)))
    up = _rnd(_mm(hn_sel, pltpu.bitcast(wu_ref[...], BF16)))
    act = _rnd(_rnd(gate * jax.nn.sigmoid(gate)) * up)
    y = _rnd(_mm(act, pltpu.bitcast(wd_ref[...], BF16)))
    y = _rnd(y * jnp.concatenate([_rnd(jax.nn.sigmoid(score))] * n_tiles, axis=1))
    new_rows = h_sel + _rnd(hn_sel + y)

    pltpu.make_async_copy(out_ref, out_hbm, out_sem).wait()
    seg_row = lax.broadcasted_iota(jnp.int32, (seg, d_model), 0)
    for n, (s, r) in enumerate(((s0, r0), (s1, r1))):
        old = out_ref[s].astype(F32)
        out_ref[s] = jnp.where(seg_row == r, new_rows[n:n + 1], old).astype(BF16)
    fix0 = pltpu.make_async_copy(out_ref.at[s0], out_hbm.at[s0], sem.at[0])
    fix1 = pltpu.make_async_copy(out_ref.at[s1], out_hbm.at[s1], sem.at[1])
    fix0.start()

    @pl.when(s0 != s1)
    def _():
        fix1.start()
        fix1.wait()

    fix0.wait()


@functools.partial(jax.jit, static_argnames=("A_seg_len",))
def pallas_sequential_preLN__memory_aug_recurrent_mem_tr__moe_arch_mod__prompt_kernel(
    A_x: jax.Array,
    A_mem0: jax.Array,
    A_Wq: jax.Array,
    A_Wk: jax.Array,
    A_Wv: jax.Array,
    A_Wo: jax.Array,
    A_seg_len: int,
    B_x: jax.Array,
    B_w_r: jax.Array,
    B_w_gate: jax.Array,
    B_w_up: jax.Array,
    B_w_down: jax.Array,
):
    del B_x
    batch, seq, d_model = A_x.shape
    n_mem = A_mem0.shape[1]
    _, n_heads, d_head = A_Wq.shape
    d_ff = B_w_gate.shape[1]
    seg = int(A_seg_len)
    n_seg = seq // seg
    assert batch == 1 and seq == n_seg * seg and seq <= 1 << 13 and n_seg % _UNROLL == 0

    hbm = pl.BlockSpec(memory_space=pl.ANY)
    out = pl.pallas_call(
        _kernel,
        out_shape=jax.ShapeDtypeStruct((n_seg, seg, d_model), A_x.dtype),
        in_specs=[hbm] * 10,
        out_specs=hbm,
        scratch_shapes=[
            pltpu.VMEM((n_mem, d_model), BF16),
            pltpu.VMEM((d_model // _LANES, _LANES), BF16),
            pltpu.VMEM((n_seg, seg, d_model), BF16),
            pltpu.VMEM((n_seg, _PRE, d_model), BF16),
            pltpu.VMEM((n_seg * _PRE // 2, d_model), U32),
            pltpu.VMEM((n_seg * _PRE, d_model), F32),
            pltpu.VMEM((3, n_heads // 2, d_model, d_head), U32),
            pltpu.VMEM((3, n_heads, d_model // 2, d_head), U32),
            pltpu.VMEM((n_heads, d_head // 2, d_model), U32),
            pltpu.VMEM((d_model // 2, d_ff), U32),
            pltpu.VMEM((d_model // 2, d_ff), U32),
            pltpu.VMEM((d_ff // 2, d_model), U32),
            pltpu.VMEM((2 * n_heads + _Q_HEADS + 1, n_seg * _PRE, d_head), F32),
            pltpu.VMEM((seg, d_model), F32),
            pltpu.VMEM((n_seg, seg, d_model), F32),
            pltpu.VMEM((n_seg, seg, d_model), F32),
            pltpu.VMEM((n_seg, seg, d_model), BF16),
            pltpu.SemaphoreType.DMA((len(_PHASES) + 4,)),
        ],
        compiler_params=pltpu.CompilerParams(vmem_limit_bytes=100 * 1024 * 1024),
        name="rmt_mod",
    )(
        A_x.reshape(n_seg, seg, d_model),
        A_mem0.reshape(n_mem, d_model),
        A_Wq, A_Wk, A_Wv, A_Wo,
        B_w_r.reshape(d_model // _LANES, _LANES),
        B_w_gate, B_w_up, B_w_down,
    )
    return out.reshape(batch, seq, d_model)
```

```python
import functools

import jax
import jax.numpy as jnp
import numpy as np
from jax import lax
import jax.experimental.pallas as pl
import jax.experimental.pallas.tpu as pltpu

F32 = jnp.float32
BF16 = jnp.bfloat16
U32 = jnp.uint32

_LANES = 128
_EPS = 1e-5
_PRE = 8
_KEY_BASE = 1 << 29
_UNROLL = 8
_Q_HEADS = 1 * _UNROLL
_RAMP = (0, 1, 3, 8)
_STEADY = 2
_LAST = 4


def _mm(a, b):
    return lax.dot_general(a, b, (((1,), (0,)), ((), ())), preferred_element_type=F32)


def _mm_t(a, b):
    return lax.dot_general(a, b, (((1,), (1,)), ((), ())), preferred_element_type=F32)


def _rnd(x):
    return x.astype(BF16).astype(F32)


def _moments(x):
    inv_n = 1.0 / x.shape[-1]
    mean = jnp.sum(x, axis=-1, keepdims=True) * inv_n
    c = x - mean
    return mean, c, jnp.sum(c * c, axis=-1, keepdims=True) * inv_n


def _layernorm(x):
    _, c, var = _moments(x)
    return c * lax.rsqrt(var + _EPS)


def _layernorm_rounded(x):
    mean, _, var = _moments(x)
    den = _rnd(jnp.sqrt(_rnd(_rnd(var) + float(np.asarray(_EPS, dtype=BF16)))))
    return _rnd(_rnd(x - _rnd(mean)) / den)


def _issue_order(n_heads, cost_a, lat_ab=200, lat_bc=480, lat_cd=200, defer=28, group=2):
    cost = dict(A=cost_a, B=10, C=10, D=40)
    width = dict(A=1, B=group, C=group, D=1)
    wait = dict(B=("A", lat_ab), C=("B", lat_bc), D=("C", lat_cd))
    nxt = dict.fromkeys(cost, 0)
    ops, done, t = [], {}, 0

    def ready(kind):
        src, lat = wait[kind]
        last = nxt[kind] + width[kind] - 1
        return last < nxt[src] and t >= done[src, last] + lat

    while nxt["D"] < n_heads:
        kind = next((c for c in "CB" if ready(c)), None)
        if kind is None and ready("D") and (nxt["A"] == n_heads or nxt["A"] - nxt["D"] > defer):
            kind = "D"
        if kind is None and nxt["A"] < n_heads:
            kind = "A"
        if kind is None:
            t += 10
            continue
        for _ in range(width[kind]):
            t += cost[kind]
            ops.append((kind, nxt[kind]))
            done[kind, nxt[kind]] = t
            nxt[kind] += 1
    return ops


def _kernel(
    x_hbm, mem0_hbm, wq_hbm, wk_hbm, wv_hbm, wo_hbm, wr_hbm, wg_hbm, wu_hbm, wd_hbm,
    out_hbm,
    mem0_ref, wr_ref, x_ref, xpre_ref, lhs_ref, lhs32_ref, stage_ref, w_ref, wo_ref, wg_ref, wu_ref, wd_ref,
    kv_ref, attn_ref, h_ref, hn_ref, out_ref, sem,
):
    n_seg, seg, d_model = x_hbm.shape
    n_mem = mem0_ref.shape[0]
    n_heads, d_head = wo_hbm.shape[0], wo_hbm.shape[1]
    n_pairs = n_heads // 2
    n_tiles = d_model // _LANES
    n_rows = seg + n_mem
    scale = float(np.asarray(d_head ** -0.5, dtype=BF16))

    w_words = [w.bitcast(U32) for w in (wq_hbm, wk_hbm, wv_hbm)]

    slot_of = (2 * n_heads, 0, n_heads)
    half = n_seg // 2
    x_head, x_rest = pl.ds(0, _UNROLL + 1), pl.ds(_UNROLL + 1, n_seg - _UNROLL - 1)

    def pair(m, i):
        return w_words[m].at[:, i, :], stage_ref.at[m, i]

    units = [(m, i) for i in range(n_pairs) for m in (1, 2)]
    ramp = [units[lo:hi] for lo, hi in zip(_RAMP, _RAMP[1:])]
    steady_pairs = (len(units) - _RAMP[-1] - _LAST) // (2 * _STEADY)

    def steady(n):
        first = _RAMP[-1] // 2 + n * steady_pairs
        return [(m, first + i) for i in range(steady_pairs) for m in (1, 2)]

    last = units[_RAMP[-1] + 2 * _STEADY * steady_pairs:]
    q_units = [(0, i) for i in range(n_pairs)]
    batches = [
        [(x_hbm.at[pl.ds(n * half, half), pl.ds(seg - _PRE, _PRE), :], xpre_ref.at[pl.ds(n * half, half)])]
        for n in range(2)
    ]
    batches += [
        [pair(m, i) for m, i in phase]
        for phase in ramp + [steady(n) for n in range(_STEADY)] + [last + q_units]
    ]
    batches[-1] += [(x_hbm.at[x_head], x_ref.at[x_head]), (mem0_hbm, mem0_ref), (wr_hbm, wr_ref)]
    batches.append([(wo_hbm.bitcast(U32), wo_ref)])
    batches.append([
        (x_hbm.at[x_rest], x_ref.at[x_rest]),
        (wg_hbm.bitcast(U32), wg_ref), (wu_hbm.bitcast(U32), wu_ref), (wd_hbm.bitcast(U32), wd_ref),
    ])
    out_sem = sem.at[len(batches)]

    def start(n):
        for src, dst in batches[n]:
            pltpu.make_async_copy(src, dst, sem.at[n]).start()

    def wait(n):
        for src, dst in batches[n]:
            pltpu.make_async_copy(src, dst, sem.at[n]).wait()

    def split_pair(m, i, after=None):
        for c in range(n_tiles):
            words = stage_ref[m, i, pl.ds(c * _LANES, _LANES), :]
            if after is not None:
                at = after.shape[0] // n_tiles * c
                words = words | ((pltpu.bitcast(after[at:at + 1], U32) >> 31) >> 1)
            for j, bits in enumerate((words, words >> 16)):
                w_ref[m, 2 * i + j, pl.ds(c * _LANES // 2, _LANES // 2), :] = pltpu.bitcast(
                    bits.astype(jnp.uint16), U32)

    state = kv_ref.at[2 * n_heads + _Q_HEADS]
    first_at, second_at = pl.ds(n_tiles * seg, 8), pl.ds(n_tiles * seg + 8, 8)

    def stage_segment(s):
        xn = _layernorm(x_ref[s].astype(F32))
        for j in range(n_tiles):
            state[pl.ds(j * seg, seg), :] = xn[:, j * _LANES:(j + 1) * _LANES]

    start(0)
    start(1)
    for n in range(2):
        wait(n)
        start(n + 2)
        xpre = xpre_ref[pl.ds(n * half, half)].astype(F32).reshape(half * _PRE, d_model)
        xpre = _layernorm(xpre)
        lhs32_ref[pl.ds(n * half * _PRE, half * _PRE), :] = xpre
        lhs_ref[pl.ds(n * half * _PRE // 2, half * _PRE // 2), :] = pltpu.bitcast(xpre.astype(BF16), U32)

    def hoist(phase, extra=()):
        for u, (m, i) in enumerate(phase):
            split_pair(m, i)
            for j in range(2):
                lhs = pltpu.bitcast(lhs_ref[...], BF16)
                y = _mm(lhs, pltpu.bitcast(w_ref[m, 2 * i + j], BF16))
                kv_ref[slot_of[m] + 2 * i + j] = y
                per = -(-len(extra) // (2 * len(phase)))
                for n, unit in enumerate(extra[(2 * u + j) * per:][:per]):
                    split_pair(*unit, after=y[n * y.shape[0] // per:(n + 1) * y.shape[0] // per])

    for n, phase in enumerate(ramp):
        wait(n + 2)
        for nxt in range(n + 4, n + 5 if phase is not ramp[-1] else len(batches) - 1):
            start(nxt)
        hoist(phase)

    def steady_body(it, _):
        for unit in steady(it):
            pltpu.make_async_copy(*pair(*unit), sem.at[len(ramp) + 2 + it]).wait()
        hoist(steady(it))

    lax.fori_loop(0, _STEADY, steady_body, None)
    wait(len(batches) - 3)
    start(len(batches) - 1)
    hoist(last, q_units)
    for t in range(_Q_HEADS):
        if t % _UNROLL:
            rows = pl.ds(0, t % _UNROLL * _PRE)
            kv_ref[slot_of[0] + t, rows, :] = _mm(lhs32_ref[rows, :], pltpu.bitcast(w_ref[0, t], BF16))
    stage_segment(0)
    attn_ref[...] = jnp.zeros((seg, d_model), F32)
    state[first_at, :] = state[second_at, :] = jnp.zeros((8, _LANES), F32)
    wait(len(batches) - 2)

    row = lax.broadcasted_iota(jnp.int32, (n_rows, n_rows), 0)
    col = lax.broadcasted_iota(jnp.int32, (n_rows, n_rows), 1)
    visible = (row >= seg) | (col >= seg) | (row >= col)
    seg_token = lax.broadcasted_iota(jnp.int32, (seg, _LANES), 0)
    token_bits = (n_seg * seg - 1).bit_length()
    token_mask = (1 << token_bits) - 1
    w_route = wr_ref[...].astype(F32)
    order = _issue_order(n_heads, cost_a=n_rows + 2 * (n_rows - _PRE))
    at = order.index(("A", 4))
    order[at:at] = [("F", 0), ("N", 0)]

    def routing_key(hn, s):
        prod = hn[:, :_LANES] * w_route[0:1]
        for j in range(1, n_tiles):
            prod = prod + hn[:, j * _LANES:(j + 1) * _LANES] * w_route[j:j + 1]
        r = jnp.broadcast_to(_rnd(jnp.sum(prod, axis=-1, keepdims=True)), (seg, _LANES))
        bits = pltpu.bitcast(r, jnp.int32) >> 16
        rank = jnp.where(bits < 0, ~bits, bits + 0x8000)
        rank = jnp.where(r == 0.0, 0x8000, jnp.where(r == r, rank, 0))
        key = _KEY_BASE + (rank << token_bits) + (token_mask - s * seg - seg_token)
        return pltpu.bitcast(key, F32)

    def finish_segment(s, live=True):
        h = _rnd(x_ref[s].astype(F32) + _rnd(attn_ref[...]))
        hn = _layernorm_rounded(h)
        h_ref[s] = h
        hn_ref[s] = hn
        out_ref[s] = (h + hn).astype(BF16)
        key = jnp.where(live, routing_key(hn, s), 0.0)
        first, second = state[first_at, :], state[second_at, :]
        for j in range(0, seg, 8):
            second = jnp.maximum(second, jnp.minimum(first, key[j:j + 8]))
            first = jnp.maximum(first, key[j:j + 8])
        state[first_at, :], state[second_at, :] = first, second

    def attend(s, turn, mem):
        xn = jnp.concatenate([state[pl.ds(j * seg, seg), :] for j in range(n_tiles)], axis=1)
        own = seg - _PRE
        pre = pl.ds(pl.multiple_of(s * _PRE, _PRE), _PRE)
        heads = [(turn + t) % _UNROLL for t in range(_UNROLL)] + list(range(_UNROLL, n_heads))

        first = jnp.minimum(s, n_seg - _UNROLL)
        ahead = pl.ds(pl.multiple_of(first * _PRE, _PRE), _UNROLL * _PRE)
        for t in range(_UNROLL + turn, _Q_HEADS, _UNROLL):
            kv_ref[slot_of[0] + t, ahead, :] = _mm(lhs32_ref[ahead, :], pltpu.bitcast(w_ref[0, t], BF16))

        def project(m, t):
            w = pltpu.bitcast(w_ref[m, heads[t]], BF16)
            if m == 0 and t >= _Q_HEADS:
                return _mm(jnp.concatenate([xn, mem], axis=0), w)
            if m == 0 and t == 0:
                y = _mm(jnp.concatenate([xn[:own], lhs32_ref[ahead, :], mem], axis=0), w)
                kv_ref[slot_of[m] + heads[t], ahead, :] = y[own:-n_mem]
            else:
                y = _mm(jnp.concatenate([xn[:own], mem], axis=0), w)
            return jnp.concatenate(
                [y[:own], kv_ref[slot_of[m] + heads[t], pre, :], y[-n_mem:]], axis=0)

        q, k, v, p, o = {}, {}, {}, {}, {}
        acc = [None] * n_tiles
        for kind, t in order:
            if kind == "A":
                q[t] = project(0, t)
                k[t] = project(1, t).astype(BF16)
                v[t] = project(2, t).astype(BF16)
            elif kind == "B":
                sc = jnp.where(visible, _mm_t(q[t], k[t]) * scale, -1e9)
                e = jnp.exp(sc - jnp.max(sc, axis=-1, keepdims=True))
                p[t] = e / jnp.sum(e, axis=-1, keepdims=True)
            elif kind == "C":
                y = _mm(p[t], v[t])
                o[t] = jnp.concatenate([y[seg:], y[:seg]], axis=0)
            elif kind == "F":
                finish_segment(jnp.maximum(s - 1, 0), live=s > 0)
            elif kind == "N":
                stage_segment(jnp.minimum(s + 1, n_seg - 1))
            else:
                for j in range(n_tiles):
                    w = pltpu.bitcast(wo_ref[heads[t], :, j * _LANES:(j + 1) * _LANES], BF16)
                    y = _mm(o[t], w)
                    acc[j] = y if acc[j] is None else acc[j] + y
        y = jnp.concatenate(acc, axis=1)
        attn_ref[...] = y[n_mem:]
        return _rnd(y[:n_mem])

    def seg_body(it, mem):
        @pl.when(it == 1)
        def _():
            wait(len(batches) - 1)

        @pl.when(it == n_iter - 1)
        def _():
            blk = pl.ds(0, n_seg - _UNROLL - 1)
            pltpu.make_async_copy(out_ref.at[blk], out_hbm.at[blk], out_sem).start()

        for u in range(_UNROLL):
            mem = attend(it * _UNROLL + u, u, mem)
        return mem

    n_iter = n_seg // _UNROLL
    lax.fori_loop(0, n_iter, seg_body, mem0_ref[...].astype(F32))
    finish_segment(n_seg - 1)
    blk = pl.ds(n_seg - _UNROLL - 1, _UNROLL + 1)
    pltpu.make_async_copy(out_ref.at[blk], out_hbm.at[blk], out_sem).start()

    first, second = state[first_at, :], state[second_at, :]
    best = jnp.max(first, axis=0, keepdims=True)
    runner_up = jnp.max(jnp.where(first == best, second, first), axis=0, keepdims=True)
    upper = lax.broadcasted_iota(jnp.int32, (8, _LANES), 0) == 0
    keys = pltpu.bitcast(jnp.where(upper, best, runner_up), jnp.int32) - _KEY_BASE
    tokens = jnp.minimum(token_mask - (keys & token_mask), n_seg * seg - 1)
    rank = keys >> token_bits
    score = pltpu.bitcast(jnp.where(rank < 0x8000, ~rank, rank - 0x8000) << 16, F32)
    (s0, r0), (s1, r1) = [(tokens[n, 0] // seg, tokens[n, 0] % seg) for n in range(2)]

    def picked(ref):
        upper = lax.broadcasted_iota(jnp.int32, (8, d_model), 0) == 0
        return jnp.where(upper, ref[s0, pl.ds(r0, 1), :], ref[s1, pl.ds(r1, 1), :])

    h_sel, hn_sel = picked(h_ref), picked(hn_ref)
    gate = _rnd(_mm(hn_sel, pltpu.bitcast(wg_ref[...], BF16)))
    up = _rnd(_mm(hn_sel, pltpu.bitcast(wu_ref[...], BF16)))
    act = _rnd(_rnd(gate * jax.nn.sigmoid(gate)) * up)
    y = _rnd(_mm(act, pltpu.bitcast(wd_ref[...], BF16)))
    y = _rnd(y * jnp.concatenate([_rnd(jax.nn.sigmoid(score))] * n_tiles, axis=1))
    new_rows = h_sel + _rnd(hn_sel + y)

    pltpu.make_async_copy(out_ref, out_hbm, out_sem).wait()
    seg_row = lax.broadcasted_iota(jnp.int32, (seg, d_model), 0)
    for n, (s, r) in enumerate(((s0, r0), (s1, r1))):
        old = out_ref[s].astype(F32)
        out_ref[s] = jnp.where(seg_row == r, new_rows[n:n + 1], old).astype(BF16)
    fix0 = pltpu.make_async_copy(out_ref.at[s0], out_hbm.at[s0], sem.at[0])
    fix1 = pltpu.make_async_copy(out_ref.at[s1], out_hbm.at[s1], sem.at[1])
    fix0.start()

    @pl.when(s0 != s1)
    def _():
        fix1.start()
        fix1.wait()

    fix0.wait()


@functools.partial(jax.jit, static_argnames=("A_seg_len",))
def pallas_sequential_preLN__memory_aug_recurrent_mem_tr__moe_arch_mod__prompt_kernel(
    A_x: jax.Array,
    A_mem0: jax.Array,
    A_Wq: jax.Array,
    A_Wk: jax.Array,
    A_Wv: jax.Array,
    A_Wo: jax.Array,
    A_seg_len: int,
    B_x: jax.Array,
    B_w_r: jax.Array,
    B_w_gate: jax.Array,
    B_w_up: jax.Array,
    B_w_down: jax.Array,
):
    del B_x
    batch, seq, d_model = A_x.shape
    n_mem = A_mem0.shape[1]
    _, n_heads, d_head = A_Wq.shape
    d_ff = B_w_gate.shape[1]
    seg = int(A_seg_len)
    n_seg = seq // seg
    assert batch == 1 and seq == n_seg * seg and seq <= 1 << 13 and n_seg % _UNROLL == 0

    hbm = pl.BlockSpec(memory_space=pl.ANY)
    out = pl.pallas_call(
        _kernel,
        out_shape=jax.ShapeDtypeStruct((n_seg, seg, d_model), A_x.dtype),
        in_specs=[hbm] * 10,
        out_specs=hbm,
        scratch_shapes=[
            pltpu.VMEM((n_mem, d_model), BF16),
            pltpu.VMEM((d_model // _LANES, _LANES), BF16),
            pltpu.VMEM((n_seg, seg, d_model), BF16),
            pltpu.VMEM((n_seg, _PRE, d_model), BF16),
            pltpu.VMEM((n_seg * _PRE // 2, d_model), U32),
            pltpu.VMEM((n_seg * _PRE, d_model), F32),
            pltpu.VMEM((3, n_heads // 2, d_model, d_head), U32),
            pltpu.VMEM((3, n_heads, d_model // 2, d_head), U32),
            pltpu.VMEM((n_heads, d_head // 2, d_model), U32),
            pltpu.VMEM((d_model // 2, d_ff), U32),
            pltpu.VMEM((d_model // 2, d_ff), U32),
            pltpu.VMEM((d_ff // 2, d_model), U32),
            pltpu.VMEM((2 * n_heads + _Q_HEADS + 1, n_seg * _PRE, d_head), F32),
            pltpu.VMEM((seg, d_model), F32),
            pltpu.VMEM((n_seg, seg, d_model), F32),
            pltpu.VMEM((n_seg, seg, d_model), F32),
            pltpu.VMEM((n_seg, seg, d_model), BF16),
            pltpu.SemaphoreType.DMA((len(_RAMP) + _STEADY + 5,)),
        ],
        compiler_params=pltpu.CompilerParams(vmem_limit_bytes=100 * 1024 * 1024),
        name="rmt_mod",
    )(
        A_x.reshape(n_seg, seg, d_model),
        A_mem0.reshape(n_mem, d_model),
        A_Wq, A_Wk, A_Wv, A_Wo,
        B_w_r.reshape(d_model // _LANES, _LANES),
        B_w_gate, B_w_up, B_w_down,
    )
    return out.reshape(batch, seq, d_model)
```

```python
import functools

import jax
import jax.numpy as jnp
import numpy as np
from jax import lax
import jax.experimental.pallas as pl
import jax.experimental.pallas.tpu as pltpu

F32 = jnp.float32
BF16 = jnp.bfloat16
U32 = jnp.uint32

_LANES = 128
_EPS = 1e-5
_PRE = 8
_KEY_BASE = 1 << 29
_UNROLL = 8
_Q_HEADS = 1 * _UNROLL
_RAMP = (0, 1, 3, 8)
_STEADY = 2
_LAST = 4


def _mm(a, b):
    return lax.dot_general(a, b, (((1,), (0,)), ((), ())), preferred_element_type=F32)


def _mm_t(a, b):
    return lax.dot_general(a, b, (((1,), (1,)), ((), ())), preferred_element_type=F32)


def _rnd(x):
    return x.astype(BF16).astype(F32)


def _moments(x):
    inv_n = 1.0 / x.shape[-1]
    mean = jnp.sum(x, axis=-1, keepdims=True) * inv_n
    c = x - mean
    return mean, c, jnp.sum(c * c, axis=-1, keepdims=True) * inv_n


def _layernorm(x):
    _, c, var = _moments(x)
    return c * lax.rsqrt(var + _EPS)


def _layernorm_rounded(x):
    mean, _, var = _moments(x)
    den = _rnd(jnp.sqrt(_rnd(_rnd(var) + float(np.asarray(_EPS, dtype=BF16)))))
    return _rnd(_rnd(x - _rnd(mean)) / den)


def _issue_order(n_heads, cost_a, lat_ab=200, lat_bc=480, lat_cd=200, defer=28, group=2):
    cost = dict(A=cost_a, B=10, C=10, D=40)
    width = dict(A=1, B=group, C=group, D=1)
    wait = dict(B=("A", lat_ab), C=("B", lat_bc), D=("C", lat_cd))
    nxt = dict.fromkeys(cost, 0)
    ops, done, t = [], {}, 0

    def ready(kind):
        src, lat = wait[kind]
        last = nxt[kind] + width[kind] - 1
        return last < nxt[src] and t >= done[src, last] + lat

    while nxt["D"] < n_heads:
        kind = next((c for c in "CB" if ready(c)), None)
        if kind is None and ready("D") and (nxt["A"] == n_heads or nxt["A"] - nxt["D"] > defer):
            kind = "D"
        if kind is None and nxt["A"] < n_heads:
            kind = "A"
        if kind is None:
            t += 10
            continue
        for _ in range(width[kind]):
            t += cost[kind]
            ops.append((kind, nxt[kind]))
            done[kind, nxt[kind]] = t
            nxt[kind] += 1
    return ops


def _kernel(
    x_hbm, mem0_hbm, wq_hbm, wk_hbm, wv_hbm, wo_hbm, wr_hbm, wg_hbm, wu_hbm, wd_hbm,
    out_hbm,
    mem0_ref, wr_ref, x_ref, xpre_ref, lhs_ref, lhs32_ref, stage_ref, w_ref, wo_ref, wg_ref, wu_ref, wd_ref,
    kv_ref, attn_ref, h_ref, hn_ref, out_ref, sem,
):
    n_seg, seg, d_model = x_hbm.shape
    n_mem = mem0_ref.shape[0]
    n_heads, d_head = wo_hbm.shape[0], wo_hbm.shape[1]
    n_pairs = n_heads // 2
    n_tiles = d_model // _LANES
    n_rows = seg + n_mem
    scale = float(np.asarray(d_head ** -0.5, dtype=BF16))

    w_words = [w.bitcast(U32) for w in (wq_hbm, wk_hbm, wv_hbm)]

    slot_of = (2 * n_heads, 0, n_heads)
    half = n_seg // 2
    x_head, x_rest = pl.ds(0, _UNROLL + 1), pl.ds(_UNROLL + 1, n_seg - _UNROLL - 1)

    def pair(m, i):
        return w_words[m].at[:, i, :], stage_ref.at[m, i]

    units = [(m, i) for i in range(n_pairs) for m in (1, 2)]
    ramp = [units[lo:hi] for lo, hi in zip(_RAMP, _RAMP[1:])]
    steady_pairs = (len(units) - _RAMP[-1] - _LAST) // (2 * _STEADY)

    def steady(n):
        first = _RAMP[-1] // 2 + n * steady_pairs
        return [(m, first + i) for i in range(steady_pairs) for m in (1, 2)]

    last = units[_RAMP[-1] + 2 * _STEADY * steady_pairs:]
    q_units = [(0, i) for i in range(n_pairs)]
    batches = [
        [(x_hbm.at[pl.ds(n * half, half), pl.ds(seg - _PRE, _PRE), :], xpre_ref.at[pl.ds(n * half, half)])]
        for n in range(2)
    ]
    batches += [
        [pair(m, i) for m, i in phase]
        for phase in ramp + [steady(n) for n in range(_STEADY)] + [last + q_units]
    ]
    batches[-1] += [(x_hbm.at[x_head], x_ref.at[x_head]), (mem0_hbm, mem0_ref), (wr_hbm, wr_ref)]
    batches.append([(wo_hbm.bitcast(U32), wo_ref)])
    batches.append([
        (x_hbm.at[x_rest], x_ref.at[x_rest]),
        (wg_hbm.bitcast(U32), wg_ref), (wu_hbm.bitcast(U32), wu_ref), (wd_hbm.bitcast(U32), wd_ref),
    ])
    out_sem = sem.at[len(batches)]

    def start(n):
        for src, dst in batches[n]:
            pltpu.make_async_copy(src, dst, sem.at[n]).start()

    def wait(n):
        for src, dst in batches[n]:
            pltpu.make_async_copy(src, dst, sem.at[n]).wait()

    def split_pair(m, i, after=None):
        for c in range(n_tiles):
            words = stage_ref[m, i, pl.ds(c * _LANES, _LANES), :]
            if after is not None:
                at = after.shape[0] // n_tiles * c
                words = words | ((pltpu.bitcast(after[at:at + 1], U32) >> 31) >> 1)
            for j, bits in enumerate((words, words >> 16)):
                w_ref[m, 2 * i + j, pl.ds(c * _LANES // 2, _LANES // 2), :] = pltpu.bitcast(
                    bits.astype(jnp.uint16), U32)

    state = kv_ref.at[2 * n_heads + _Q_HEADS]
    first_at, second_at = pl.ds(n_tiles * seg, 8), pl.ds(n_tiles * seg + 8, 8)

    def stage_segment(s):
        xn = _layernorm(x_ref[s].astype(F32))
        for j in range(n_tiles):
            state[pl.ds(j * seg, seg), :] = xn[:, j * _LANES:(j + 1) * _LANES]

    start(0)
    start(1)
    for n in range(2):
        wait(n)
        start(n + 2)
        xpre = xpre_ref[pl.ds(n * half, half)].astype(F32).reshape(half * _PRE, d_model)
        xpre = _layernorm(xpre)
        lhs32_ref[pl.ds(n * half * _PRE, half * _PRE), :] = xpre
        lhs_ref[pl.ds(n * half * _PRE // 2, half * _PRE // 2), :] = pltpu.bitcast(xpre.astype(BF16), U32)

    def hoist(phase, extra=()):
        for u, (m, i) in enumerate(phase):
            split_pair(m, i)
            for j in range(2):
                lhs = pltpu.bitcast(lhs_ref[...], BF16)
                y = _mm(lhs, pltpu.bitcast(w_ref[m, 2 * i + j], BF16))
                kv_ref[slot_of[m] + 2 * i + j] = y
                per = -(-len(extra) // (2 * len(phase)))
                for n, unit in enumerate(extra[(2 * u + j) * per:][:per]):
                    split_pair(*unit, after=y[n * y.shape[0] // per:(n + 1) * y.shape[0] // per])

    for n, phase in enumerate(ramp):
        wait(n + 2)
        for nxt in range(n + 4, n + 5 if phase is not ramp[-1] else len(batches) - 1):
            start(nxt)
        hoist(phase)

    def steady_body(it, _):
        for unit in steady(it):
            pltpu.make_async_copy(*pair(*unit), sem.at[len(ramp) + 2 + it]).wait()
        hoist(steady(it))

    lax.fori_loop(0, _STEADY, steady_body, None)
    wait(len(batches) - 3)
    start(len(batches) - 1)
    hoist(last, q_units)
    for t in range(_Q_HEADS):
        if t % _UNROLL:
            rows = pl.ds(0, t % _UNROLL * _PRE)
            kv_ref[slot_of[0] + t, rows, :] = _mm(lhs32_ref[rows, :], pltpu.bitcast(w_ref[0, t], BF16))
    stage_segment(0)
    attn_ref[...] = jnp.zeros((seg, d_model), F32)
    state[first_at, :] = state[second_at, :] = jnp.zeros((8, _LANES), F32)
    wait(len(batches) - 2)

    row = lax.broadcasted_iota(jnp.int32, (n_rows, n_rows), 0)
    col = lax.broadcasted_iota(jnp.int32, (n_rows, n_rows), 1)
    visible = (row >= seg) | (col >= seg) | (row >= col)
    seg_token = lax.broadcasted_iota(jnp.int32, (seg, _LANES), 0)
    token_bits = (n_seg * seg - 1).bit_length()
    token_mask = (1 << token_bits) - 1
    w_route = wr_ref[...].astype(F32)
    order = _issue_order(n_heads, cost_a=n_rows + 2 * (n_rows - _PRE))
    at = order.index(("A", 6))
    order.insert(at, ("F", 0))
    order.append(("N", 0))

    def routing_key(hn, s):
        prod = hn[:, :_LANES] * w_route[0:1]
        for j in range(1, n_tiles):
            prod = prod + hn[:, j * _LANES:(j + 1) * _LANES] * w_route[j:j + 1]
        r = jnp.broadcast_to(_rnd(jnp.sum(prod, axis=-1, keepdims=True)), (seg, _LANES))
        bits = pltpu.bitcast(r, jnp.int32) >> 16
        rank = jnp.where(bits < 0, ~bits, bits + 0x8000)
        rank = jnp.where(r == 0.0, 0x8000, jnp.where(r == r, rank, 0))
        key = _KEY_BASE + (rank << token_bits) + (token_mask - s * seg - seg_token)
        return pltpu.bitcast(key, F32)

    def finish_segment(s, live=True):
        h = _rnd(x_ref[s].astype(F32) + _rnd(attn_ref[...]))
        hn = _layernorm_rounded(h)
        h_ref[s] = h
        hn_ref[s] = hn
        out_ref[s] = (h + hn).astype(BF16)
        key = jnp.where(live, routing_key(hn, s), 0.0)
        first, second = state[first_at, :], state[second_at, :]
        for j in range(0, seg, 8):
            second = jnp.maximum(second, jnp.minimum(first, key[j:j + 8]))
            first = jnp.maximum(first, key[j:j + 8])
        state[first_at, :], state[second_at, :] = first, second

    def attend(s, turn, mem):
        xn = jnp.concatenate([state[pl.ds(j * seg, seg), :] for j in range(n_tiles)], axis=1)
        own = seg - _PRE
        pre = pl.ds(pl.multiple_of(s * _PRE, _PRE), _PRE)
        heads = [(turn + t) % _UNROLL for t in range(_UNROLL)] + list(range(_UNROLL, n_heads))

        first = jnp.minimum(s, n_seg - _UNROLL)
        ahead = pl.ds(pl.multiple_of(first * _PRE, _PRE), _UNROLL * _PRE)
        for t in range(_UNROLL + turn, _Q_HEADS, _UNROLL):
            kv_ref[slot_of[0] + t, ahead, :] = _mm(lhs32_ref[ahead, :], pltpu.bitcast(w_ref[0, t], BF16))

        short = jnp.concatenate([xn[:own], mem], axis=0).astype(BF16)

        def project(m, t):
            w = pltpu.bitcast(w_ref[m, heads[t]], BF16)
            if m == 0 and t >= _Q_HEADS:
                return _mm(jnp.concatenate([xn, mem], axis=0), w)
            if m == 0 and t == 0:
                y = _mm(jnp.concatenate([xn[:own], lhs32_ref[ahead, :], mem], axis=0), w)
                kv_ref[slot_of[m] + heads[t], ahead, :] = y[own:-n_mem]
            else:
                y = _mm(short, w)
            return jnp.concatenate(
                [y[:own], kv_ref[slot_of[m] + heads[t], pre, :], y[-n_mem:]], axis=0)

        q, k, v, p, o = {}, {}, {}, {}, {}
        acc = [None] * n_tiles
        for kind, t in order:
            if kind == "A":
                q[t] = project(0, t)
                k[t] = project(1, t).astype(BF16)
                v[t] = project(2, t).astype(BF16)
            elif kind == "B":
                sc = jnp.where(visible, _mm_t(q[t], k[t]) * scale, -1e9)
                e = jnp.exp(sc - jnp.max(sc, axis=-1, keepdims=True))
                p[t] = e / jnp.sum(e, axis=-1, keepdims=True)
            elif kind == "C":
                y = _mm(p[t], v[t])
                o[t] = jnp.concatenate([y[seg:], y[:seg]], axis=0)
            elif kind == "F":
                finish_segment(jnp.maximum(s - 1, 0), live=s > 0)
            elif kind == "N":
                stage_segment(jnp.minimum(s + 1, n_seg - 1))
            else:
                for j in range(n_tiles):
                    w = pltpu.bitcast(wo_ref[heads[t], :, j * _LANES:(j + 1) * _LANES], BF16)
                    y = _mm(o[t], w)
                    acc[j] = y if acc[j] is None else acc[j] + y
        y = jnp.concatenate(acc, axis=1)
        attn_ref[...] = y[n_mem:]
        return _rnd(y[:n_mem])

    def seg_body(it, mem):
        @pl.when(it == 1)
        def _():
            wait(len(batches) - 1)

        @pl.when(it == n_iter - 1)
        def _():
            blk = pl.ds(0, n_seg - _UNROLL - 1)
            pltpu.make_async_copy(out_ref.at[blk], out_hbm.at[blk], out_sem).start()

        for u in range(_UNROLL):
            mem = attend(it * _UNROLL + u, u, mem)
        return mem

    n_iter = n_seg // _UNROLL
    lax.fori_loop(0, n_iter, seg_body, mem0_ref[...].astype(F32))
    finish_segment(n_seg - 1)
    blk = pl.ds(n_seg - _UNROLL - 1, _UNROLL + 1)
    pltpu.make_async_copy(out_ref.at[blk], out_hbm.at[blk], out_sem).start()

    first, second = state[first_at, :], state[second_at, :]
    best = jnp.max(first, axis=0, keepdims=True)
    runner_up = jnp.max(jnp.where(first == best, second, first), axis=0, keepdims=True)
    upper = lax.broadcasted_iota(jnp.int32, (8, _LANES), 0) == 0
    keys = pltpu.bitcast(jnp.where(upper, best, runner_up), jnp.int32) - _KEY_BASE
    tokens = jnp.minimum(token_mask - (keys & token_mask), n_seg * seg - 1)
    rank = keys >> token_bits
    score = pltpu.bitcast(jnp.where(rank < 0x8000, ~rank, rank - 0x8000) << 16, F32)
    (s0, r0), (s1, r1) = [(tokens[n, 0] // seg, tokens[n, 0] % seg) for n in range(2)]

    def picked(ref):
        upper = lax.broadcasted_iota(jnp.int32, (8, d_model), 0) == 0
        return jnp.where(upper, ref[s0, pl.ds(r0, 1), :], ref[s1, pl.ds(r1, 1), :])

    h_sel, hn_sel = picked(h_ref), picked(hn_ref)
    gate = _rnd(_mm(hn_sel, pltpu.bitcast(wg_ref[...], BF16)))
    up = _rnd(_mm(hn_sel, pltpu.bitcast(wu_ref[...], BF16)))
    act = _rnd(_rnd(gate * jax.nn.sigmoid(gate)) * up)
    y = _rnd(_mm(act, pltpu.bitcast(wd_ref[...], BF16)))
    y = _rnd(y * jnp.concatenate([_rnd(jax.nn.sigmoid(score))] * n_tiles, axis=1))
    new_rows = h_sel + _rnd(hn_sel + y)

    pltpu.make_async_copy(out_ref, out_hbm, out_sem).wait()
    seg_row = lax.broadcasted_iota(jnp.int32, (seg, d_model), 0)
    for n, (s, r) in enumerate(((s0, r0), (s1, r1))):
        old = out_ref[s].astype(F32)
        out_ref[s] = jnp.where(seg_row == r, new_rows[n:n + 1], old).astype(BF16)
    fix0 = pltpu.make_async_copy(out_ref.at[s0], out_hbm.at[s0], sem.at[0])
    fix1 = pltpu.make_async_copy(out_ref.at[s1], out_hbm.at[s1], sem.at[1])
    fix0.start()

    @pl.when(s0 != s1)
    def _():
        fix1.start()
        fix1.wait()

    fix0.wait()


@functools.partial(jax.jit, static_argnames=("A_seg_len",))
def pallas_sequential_preLN__memory_aug_recurrent_mem_tr__moe_arch_mod__prompt_kernel(
    A_x: jax.Array,
    A_mem0: jax.Array,
    A_Wq: jax.Array,
    A_Wk: jax.Array,
    A_Wv: jax.Array,
    A_Wo: jax.Array,
    A_seg_len: int,
    B_x: jax.Array,
    B_w_r: jax.Array,
    B_w_gate: jax.Array,
    B_w_up: jax.Array,
    B_w_down: jax.Array,
):
    del B_x
    batch, seq, d_model = A_x.shape
    n_mem = A_mem0.shape[1]
    _, n_heads, d_head = A_Wq.shape
    d_ff = B_w_gate.shape[1]
    seg = int(A_seg_len)
    n_seg = seq // seg
    assert batch == 1 and seq == n_seg * seg and seq <= 1 << 13 and n_seg % _UNROLL == 0

    hbm = pl.BlockSpec(memory_space=pl.ANY)
    out = pl.pallas_call(
        _kernel,
        out_shape=jax.ShapeDtypeStruct((n_seg, seg, d_model), A_x.dtype),
        in_specs=[hbm] * 10,
        out_specs=hbm,
        scratch_shapes=[
            pltpu.VMEM((n_mem, d_model), BF16),
            pltpu.VMEM((d_model // _LANES, _LANES), BF16),
            pltpu.VMEM((n_seg, seg, d_model), BF16),
            pltpu.VMEM((n_seg, _PRE, d_model), BF16),
            pltpu.VMEM((n_seg * _PRE // 2, d_model), U32),
            pltpu.VMEM((n_seg * _PRE, d_model), F32),
            pltpu.VMEM((3, n_heads // 2, d_model, d_head), U32),
            pltpu.VMEM((3, n_heads, d_model // 2, d_head), U32),
            pltpu.VMEM((n_heads, d_head // 2, d_model), U32),
            pltpu.VMEM((d_model // 2, d_ff), U32),
            pltpu.VMEM((d_model // 2, d_ff), U32),
            pltpu.VMEM((d_ff // 2, d_model), U32),
            pltpu.VMEM((2 * n_heads + _Q_HEADS + 1, n_seg * _PRE, d_head), F32),
            pltpu.VMEM((seg, d_model), F32),
            pltpu.VMEM((n_seg, seg, d_model), F32),
            pltpu.VMEM((n_seg, seg, d_model), F32),
            pltpu.VMEM((n_seg, seg, d_model), BF16),
            pltpu.SemaphoreType.DMA((len(_RAMP) + _STEADY + 5,)),
        ],
        compiler_params=pltpu.CompilerParams(vmem_limit_bytes=100 * 1024 * 1024),
        name="rmt_mod",
    )(
        A_x.reshape(n_seg, seg, d_model),
        A_mem0.reshape(n_mem, d_model),
        A_Wq, A_Wk, A_Wv, A_Wo,
        B_w_r.reshape(d_model // _LANES, _LANES),
        B_w_gate, B_w_up, B_w_down,
    )
    return out.reshape(batch, seq, d_model)
```

```python
import functools

import jax
import jax.numpy as jnp
import numpy as np
from jax import lax
import jax.experimental.pallas as pl
import jax.experimental.pallas.tpu as pltpu

F32 = jnp.float32
BF16 = jnp.bfloat16
U32 = jnp.uint32

_LANES = 128
_EPS = 1e-5
_PRE = 8
_KEY_BASE = 1 << 29
_UNROLL = 8
_RAMP = (0, 1, 3, 8)
_AHEAD = 3
_STEADY = 2
_LAST = 4


def _mm(a, b):
    return lax.dot_general(a, b, (((1,), (0,)), ((), ())), preferred_element_type=F32)


def _mm_t(a, b):
    return lax.dot_general(a, b, (((1,), (1,)), ((), ())), preferred_element_type=F32)


def _rnd(x):
    return x.astype(BF16).astype(F32)


def _moments(x):
    inv_n = 1.0 / x.shape[-1]
    mean = jnp.sum(x, axis=-1, keepdims=True) * inv_n
    c = x - mean
    return mean, c, jnp.sum(c * c, axis=-1, keepdims=True) * inv_n


def _layernorm(x):
    _, c, var = _moments(x)
    return c * lax.rsqrt(var + _EPS)


def _layernorm_rounded(x):
    mean, _, var = _moments(x)
    den = _rnd(jnp.sqrt(_rnd(_rnd(var) + float(np.asarray(_EPS, dtype=BF16)))))
    return _rnd(_rnd(x - _rnd(mean)) / den)


def _issue_order(n_heads, cost_a, lat_ab=200, lat_bc=480, lat_cd=200, defer=28, group=2):
    cost = dict(A=cost_a, B=10, C=10, D=40)
    width = dict(A=1, B=group, C=group, D=1)
    wait = dict(B=("A", lat_ab), C=("B", lat_bc), D=("C", lat_cd))
    nxt = dict.fromkeys(cost, 0)
    ops, done, t = [], {}, 0

    def ready(kind):
        src, lat = wait[kind]
        last = nxt[kind] + width[kind] - 1
        return last < nxt[src] and t >= done[src, last] + lat

    while nxt["D"] < n_heads:
        kind = next((c for c in "CB" if ready(c)), None)
        if kind is None and ready("D") and (nxt["A"] == n_heads or nxt["A"] - nxt["D"] > defer):
            kind = "D"
        if kind is None and nxt["A"] < n_heads:
            kind = "A"
        if kind is None:
            t += 10
            continue
        for _ in range(width[kind]):
            t += cost[kind]
            ops.append((kind, nxt[kind]))
            done[kind, nxt[kind]] = t
            nxt[kind] += 1
    return ops


def _kernel(
    x_hbm, mem0_hbm, wq_hbm, wk_hbm, wv_hbm, wo_hbm, wr_hbm, wg_hbm, wu_hbm, wd_hbm,
    out_hbm,
    mem0_ref, wr_ref, x_ref, xpre_ref, lhs_ref, lhs32_ref, stage_ref, w_ref, wo_ref,
    wg_ref, wu_ref, wd_ref, kv_ref, attn_ref, h_ref, hn_ref, out_ref, sem,
):
    n_seg, seg, d_model = x_hbm.shape
    n_mem = mem0_ref.shape[0]
    n_heads, d_head = wo_hbm.shape[0], wo_hbm.shape[1]
    n_pairs = n_heads // 2
    n_tiles = d_model // _LANES
    n_rows = seg + n_mem
    scale = float(np.asarray(d_head ** -0.5, dtype=BF16))

    w_words = [w.bitcast(U32) for w in (wq_hbm, wk_hbm, wv_hbm)]

    slot_of = (2 * n_heads, 0, n_heads)
    half = n_seg // 2
    x_head, x_rest = pl.ds(0, _UNROLL + 1), pl.ds(_UNROLL + 1, n_seg - _UNROLL - 1)

    def pair(m, i):
        return w_words[m].at[:, i, :], stage_ref.at[m, i]

    units = [(m, i) for i in range(n_pairs) for m in (1, 2)]
    ramp = [units[lo:hi] for lo, hi in zip(_RAMP, _RAMP[1:])]
    steady_pairs = (len(units) - _RAMP[-1] - _LAST) // (2 * _STEADY)

    def steady(n):
        first = _RAMP[-1] // 2 + n * steady_pairs
        return [(m, first + i) for i in range(steady_pairs) for m in (1, 2)]

    last = units[_RAMP[-1] + 2 * _STEADY * steady_pairs:]
    q_units = [(0, i) for i in range(n_pairs)]
    batches = [
        [(x_hbm.at[pl.ds(n * half, half), pl.ds(seg - _PRE, _PRE), :], xpre_ref.at[pl.ds(n * half, half)])]
        for n in range(2)
    ]
    batches += [
        [pair(m, i) for m, i in phase]
        for phase in ramp + [steady(n) for n in range(_STEADY)] + [last + q_units]
    ]
    batches[-1] += [(x_hbm.at[x_head], x_ref.at[x_head]), (mem0_hbm, mem0_ref), (wr_hbm, wr_ref)]
    batches.append([(wo_hbm.bitcast(U32), wo_ref)])
    batches.append([
        (x_hbm.at[x_rest], x_ref.at[x_rest]),
        (wg_hbm.bitcast(U32), wg_ref), (wu_hbm.bitcast(U32), wu_ref), (wd_hbm.bitcast(U32), wd_ref),
    ])
    out_sem = sem.at[len(batches)]

    def start(n):
        for src, dst in batches[n]:
            pltpu.make_async_copy(src, dst, sem.at[n]).start()

    def wait(n):
        for src, dst in batches[n]:
            pltpu.make_async_copy(src, dst, sem.at[n]).wait()

    def split_pair(m, i, after=None):
        for c in range(n_tiles):
            words = stage_ref[m, i, pl.ds(c * _LANES, _LANES), :]
            if after is not None:
                at = after.shape[0] // n_tiles * c
                words = words | ((pltpu.bitcast(after[at:at + 1], U32) >> 31) >> 1)
            for j, bits in enumerate((words, words >> 16)):
                w_ref[m, 2 * i + j, pl.ds(c * _LANES // 2, _LANES // 2), :] = pltpu.bitcast(
                    bits.astype(jnp.uint16), U32)

    state = kv_ref.at[2 * n_heads + _UNROLL]
    first_at, second_at = pl.ds(n_tiles * seg, 8), pl.ds(n_tiles * seg + 8, 8)

    def stage_segment(s):
        xn = _layernorm(x_ref[s].astype(F32))
        for j in range(n_tiles):
            state[pl.ds(j * seg, seg), :] = xn[:, j * _LANES:(j + 1) * _LANES]

    for n in range(_AHEAD):
        start(n)
    for n in range(2):
        wait(n)
        start(n + _AHEAD)
        xpre = xpre_ref[pl.ds(n * half, half)].astype(F32).reshape(half * _PRE, d_model)
        xpre = _layernorm(xpre)
        lhs32_ref[pl.ds(n * half * _PRE, half * _PRE), :] = xpre
        lhs_ref[pl.ds(n * half * _PRE // 2, half * _PRE // 2), :] = pltpu.bitcast(xpre.astype(BF16), U32)

    def hoist(phase, extra=()):
        for u, (m, i) in enumerate(phase):
            split_pair(m, i)
            for j in range(2):
                lhs = pltpu.bitcast(lhs_ref[...], BF16)
                y = _mm(lhs, pltpu.bitcast(w_ref[m, 2 * i + j], BF16))
                kv_ref[slot_of[m] + 2 * i + j] = y
                per = -(-len(extra) // (2 * len(phase)))
                for n, unit in enumerate(extra[(2 * u + j) * per:][:per]):
                    split_pair(*unit, after=y[n * y.shape[0] // per:(n + 1) * y.shape[0] // per])

    for n, phase in enumerate(ramp):
        wait(n + 2)
        for nxt in range(n + 2 + _AHEAD, n + 3 + _AHEAD if phase is not ramp[-1] else len(batches) - 1):
            start(nxt)
        hoist(phase)

    def steady_body(it, _):
        for unit in steady(it):
            pltpu.make_async_copy(*pair(*unit), sem.at[len(ramp) + 2 + it]).wait()
        hoist(steady(it))

    lax.fori_loop(0, _STEADY, steady_body, None)
    wait(len(batches) - 3)
    start(len(batches) - 1)
    hoist(last, q_units)
    for t in range(1, _UNROLL):
        rows = pl.ds(0, t * _PRE)
        kv_ref[slot_of[0] + t, rows, :] = _mm(lhs32_ref[rows, :], pltpu.bitcast(w_ref[0, t], BF16))
    stage_segment(0)
    attn_ref[...] = jnp.zeros((seg, d_model), F32)
    state[first_at, :] = state[second_at, :] = jnp.zeros((8, _LANES), F32)
    wait(len(batches) - 2)

    row = lax.broadcasted_iota(jnp.int32, (n_rows, n_rows), 0)
    col = lax.broadcasted_iota(jnp.int32, (n_rows, n_rows), 1)
    visible = (row >= seg) | (col >= seg) | (row >= col)
    seg_token = lax.broadcasted_iota(jnp.int32, (seg, _LANES), 0)
    token_bits = (n_seg * seg - 1).bit_length()
    token_mask = (1 << token_bits) - 1
    w_route = wr_ref[...].astype(F32)
    order = _issue_order(n_heads, cost_a=n_rows + 2 * (n_rows - _PRE))
    at = order.index(("A", 6))
    order.insert(at, ("F", 0))
    order.append(("N", 0))

    def routing_key(hn, s):
        prod = hn[:, :_LANES] * w_route[0:1]
        for j in range(1, n_tiles):
            prod = prod + hn[:, j * _LANES:(j + 1) * _LANES] * w_route[j:j + 1]
        r = jnp.broadcast_to(_rnd(jnp.sum(prod, axis=-1, keepdims=True)), (seg, _LANES))
        bits = pltpu.bitcast(r, jnp.int32) >> 16
        rank = jnp.where(bits < 0, ~bits, bits + 0x8000)
        rank = jnp.where(r == 0.0, 0x8000, jnp.where(r == r, rank, 0))
        key = _KEY_BASE + (rank << token_bits) + (token_mask - s * seg - seg_token)
        return pltpu.bitcast(key, F32)

    def finish_segment(s, live=True):
        h = _rnd(x_ref[s].astype(F32) + _rnd(attn_ref[...]))
        hn = _layernorm_rounded(h)
        h_ref[s] = h
        hn_ref[s] = hn
        out_ref[s] = (h + hn).astype(BF16)
        key = jnp.where(live, routing_key(hn, s), 0.0)
        first, second = state[first_at, :], state[second_at, :]
        for j in range(0, seg, 8):
            second = jnp.maximum(second, jnp.minimum(first, key[j:j + 8]))
            first = jnp.maximum(first, key[j:j + 8])
        state[first_at, :], state[second_at, :] = first, second

    def attend(s, turn, mem):
        xn = jnp.concatenate([state[pl.ds(j * seg, seg), :] for j in range(n_tiles)], axis=1)
        own = seg - _PRE
        pre = pl.ds(pl.multiple_of(s * _PRE, _PRE), _PRE)
        heads = [(turn + t) % _UNROLL for t in range(_UNROLL)] + list(range(_UNROLL, n_heads))

        first = jnp.minimum(s, n_seg - _UNROLL)
        ahead = pl.ds(pl.multiple_of(first * _PRE, _PRE), _UNROLL * _PRE)

        short = jnp.concatenate([xn[:own], mem], axis=0).astype(BF16)

        def project(m, t):
            w = pltpu.bitcast(w_ref[m, heads[t]], BF16)
            if m == 0 and heads[t] >= _UNROLL:
                return _mm(jnp.concatenate([xn, mem], axis=0), w)
            if m == 0 and t == 0:
                y = _mm(jnp.concatenate([xn[:own], lhs32_ref[ahead, :], mem], axis=0), w)
                kv_ref[slot_of[m] + heads[t], ahead, :] = y[own:-n_mem]
            else:
                y = _mm(short, w)
            return jnp.concatenate(
                [y[:own], kv_ref[slot_of[m] + heads[t], pre, :], y[-n_mem:]], axis=0)

        q, k, v, p, o = {}, {}, {}, {}, {}
        acc = [None] * n_tiles
        for kind, t in order:
            if kind == "A":
                q[t] = project(0, t)
                k[t] = project(1, t).astype(BF16)
                v[t] = project(2, t).astype(BF16)
            elif kind == "B":
                sc = jnp.where(visible, _mm_t(q[t], k[t]) * scale, -1e9)
                e = jnp.exp(sc - jnp.max(sc, axis=-1, keepdims=True))
                p[t] = e / jnp.sum(e, axis=-1, keepdims=True)
            elif kind == "C":
                y = _mm(p[t], v[t])
                o[t] = jnp.concatenate([y[seg:], y[:seg]], axis=0)
            elif kind == "F":
                finish_segment(jnp.maximum(s - 1, 0), live=s > 0)
            elif kind == "N":
                stage_segment(jnp.minimum(s + 1, n_seg - 1))
            else:
                for j in range(n_tiles):
                    w = pltpu.bitcast(wo_ref[heads[t], :, j * _LANES:(j + 1) * _LANES], BF16)
                    y = _mm(o[t], w)
                    acc[j] = y if acc[j] is None else acc[j] + y
        y = jnp.concatenate(acc, axis=1)
        attn_ref[...] = y[n_mem:]
        return _rnd(y[:n_mem])

    def seg_body(it, mem):
        @pl.when(it == 1)
        def _():
            wait(len(batches) - 1)

        @pl.when(it == n_iter - 1)
        def _():
            blk = pl.ds(0, n_seg - _UNROLL - 1)
            pltpu.make_async_copy(out_ref.at[blk], out_hbm.at[blk], out_sem).start()

        for u in range(_UNROLL):
            mem = attend(it * _UNROLL + u, u, mem)
        return mem

    n_iter = n_seg // _UNROLL
    lax.fori_loop(0, n_iter, seg_body, mem0_ref[...].astype(F32))
    finish_segment(n_seg - 1)
    blk = pl.ds(n_seg - _UNROLL - 1, _UNROLL + 1)
    pltpu.make_async_copy(out_ref.at[blk], out_hbm.at[blk], out_sem).start()

    first, second = state[first_at, :], state[second_at, :]
    best = jnp.max(first, axis=0, keepdims=True)
    runner_up = jnp.max(jnp.where(first == best, second, first), axis=0, keepdims=True)
    upper = lax.broadcasted_iota(jnp.int32, (8, _LANES), 0) == 0
    keys = pltpu.bitcast(jnp.where(upper, best, runner_up), jnp.int32) - _KEY_BASE
    tokens = jnp.minimum(token_mask - (keys & token_mask), n_seg * seg - 1)
    rank = keys >> token_bits
    score = pltpu.bitcast(jnp.where(rank < 0x8000, ~rank, rank - 0x8000) << 16, F32)
    (s0, r0), (s1, r1) = [(tokens[n, 0] // seg, tokens[n, 0] % seg) for n in range(2)]

    def picked(ref):
        upper = lax.broadcasted_iota(jnp.int32, (8, d_model), 0) == 0
        return jnp.where(upper, ref[s0, pl.ds(r0, 1), :], ref[s1, pl.ds(r1, 1), :])

    h_sel, hn_sel = picked(h_ref), picked(hn_ref)
    gate = _rnd(_mm(hn_sel, pltpu.bitcast(wg_ref[...], BF16)))
    up = _rnd(_mm(hn_sel, pltpu.bitcast(wu_ref[...], BF16)))
    act = _rnd(_rnd(gate * jax.nn.sigmoid(gate)) * up)
    y = _rnd(_mm(act, pltpu.bitcast(wd_ref[...], BF16)))
    y = _rnd(y * jnp.concatenate([_rnd(jax.nn.sigmoid(score))] * n_tiles, axis=1))
    new_rows = h_sel + _rnd(hn_sel + y)

    pltpu.make_async_copy(out_ref, out_hbm, out_sem).wait()
    seg_row = lax.broadcasted_iota(jnp.int32, (seg, d_model), 0)
    for n, (s, r) in enumerate(((s0, r0), (s1, r1))):
        old = out_ref[s].astype(F32)
        out_ref[s] = jnp.where(seg_row == r, new_rows[n:n + 1], old).astype(BF16)
    fix0 = pltpu.make_async_copy(out_ref.at[s0], out_hbm.at[s0], sem.at[0])
    fix1 = pltpu.make_async_copy(out_ref.at[s1], out_hbm.at[s1], sem.at[1])
    fix0.start()

    @pl.when(s0 != s1)
    def _():
        fix1.start()
        fix1.wait()

    fix0.wait()


@functools.partial(jax.jit, static_argnames=("A_seg_len",))
def pallas_sequential_preLN__memory_aug_recurrent_mem_tr__moe_arch_mod__prompt_kernel(
    A_x: jax.Array,
    A_mem0: jax.Array,
    A_Wq: jax.Array,
    A_Wk: jax.Array,
    A_Wv: jax.Array,
    A_Wo: jax.Array,
    A_seg_len: int,
    B_x: jax.Array,
    B_w_r: jax.Array,
    B_w_gate: jax.Array,
    B_w_up: jax.Array,
    B_w_down: jax.Array,
):
    del B_x
    batch, seq, d_model = A_x.shape
    n_mem = A_mem0.shape[1]
    _, n_heads, d_head = A_Wq.shape
    d_ff = B_w_gate.shape[1]
    seg = int(A_seg_len)
    n_seg = seq // seg
    assert batch == 1 and seq == n_seg * seg and seq <= 1 << 13 and d_head == _LANES
    assert n_seg % _UNROLL == 0 and n_seg * _PRE >= d_model // _LANES * seg + 16

    hbm = pl.BlockSpec(memory_space=pl.ANY)
    out = pl.pallas_call(
        _kernel,
        out_shape=jax.ShapeDtypeStruct((n_seg, seg, d_model), A_x.dtype),
        in_specs=[hbm] * 10,
        out_specs=hbm,
        scratch_shapes=[
            pltpu.VMEM((n_mem, d_model), BF16),
            pltpu.VMEM((d_model // _LANES, _LANES), BF16),
            pltpu.VMEM((n_seg, seg, d_model), BF16),
            pltpu.VMEM((n_seg, _PRE, d_model), BF16),
            pltpu.VMEM((n_seg * _PRE // 2, d_model), U32),
            pltpu.VMEM((n_seg * _PRE, d_model), F32),
            pltpu.VMEM((3, n_heads // 2, d_model, d_head), U32),
            pltpu.VMEM((3, n_heads, d_model // 2, d_head), U32),
            pltpu.VMEM((n_heads, d_head // 2, d_model), U32),
            pltpu.VMEM((d_model // 2, d_ff), U32),
            pltpu.VMEM((d_model // 2, d_ff), U32),
            pltpu.VMEM((d_ff // 2, d_model), U32),
            pltpu.VMEM((2 * n_heads + _UNROLL + 1, n_seg * _PRE, d_head), F32),
            pltpu.VMEM((seg, d_model), F32),
            pltpu.VMEM((n_seg, seg, d_model), F32),
            pltpu.VMEM((n_seg, seg, d_model), F32),
            pltpu.VMEM((n_seg, seg, d_model), BF16),
            pltpu.SemaphoreType.DMA((len(_RAMP) + _STEADY + 5,)),
        ],
        compiler_params=pltpu.CompilerParams(vmem_limit_bytes=100 * 1024 * 1024),
        name="rmt_mod",
    )(
        A_x.reshape(n_seg, seg, d_model),
        A_mem0.reshape(n_mem, d_model),
        A_Wq, A_Wk, A_Wv, A_Wo,
        B_w_r.reshape(d_model // _LANES, _LANES),
        B_w_gate, B_w_up, B_w_down,
    )
    return out.reshape(batch, seq, d_model)
```
